```python
import jax
import jax.numpy as jnp

def _softmax(x, axis=-1):
    return jax.nn.softmax(x, axis=axis)
def _gelu(x):
    return jax.nn.gelu(x, approximate=True)
def _silu(x):
    return jax.nn.silu(x)
def _sigmoid(x):
    return jax.nn.sigmoid(x)
def _layernorm(x, axis=-1, eps=1e-5):
    m = jnp.mean(x, axis=axis, keepdims=True)
    v = jnp.var(x, axis=axis, keepdims=True)
    return (x - m) / jnp.sqrt(v + eps)
def _scatter_add(tgt, idx, src, axis=0):
    return tgt.at[idx].add(src)
def _segment_sum(src, seg, n):
    return jax.ops.segment_sum(src, seg, n)
class _Rng:
    def __init__(self, key):
        self._k = key
    def _next(self):
        self._k, sub = jax.random.split(self._k)
        return sub
    def normal(self, shape):
        return jax.random.normal(self._next(), shape, dtype=jnp.bfloat16)
    def randint(self, lo, hi, shape):
        return jax.random.randint(self._next(), shape, lo, hi, dtype=jnp.int32)
    def uniform(self, shape, lo=0.0, hi=1.0):
        return jax.random.uniform(self._next(), shape, jnp.bfloat16, lo, hi)
    def permutation(self, n):
        return jax.random.permutation(self._next(), n)


kernel_name = 'interleave_layers__sliding_block__moe_arch_mod__prompt'

def setup_inputs():
    _rng = _Rng(jax.random.key(int.from_bytes(__import__("os").urandom(4), "little")))
    _w = (lambda a: (lambda t: t.astype(jnp.bfloat16) if jnp.issubdtype(t.dtype, jnp.floating) else t)(jnp.asarray(a)))
    def _A_setup():
        B, S, D = 1, 2048, 1024
        return {
            "x": _w((lambda *s: _rng.normal(s) * 0.05)(B, S, D)),
            "wqkv": _w((lambda *s: _rng.normal(s) * 0.05)(D, 3 * D)),
            "wo": _w((lambda *s: _rng.normal(s) * 0.05)(D, D)),
        }
    _A_in = _A_setup()

    def _B_setup():
        B, S, D, F, C = 1, 2048, 1024, 3584, 1
        return {
            "x": _w((lambda *s: _rng.normal(s) * 0.05)(B, S, D)),
            "w_r": _w((lambda *s: _rng.normal(s) * 0.05)(D)),
            "w_gate": _w((lambda *s: _rng.normal(s) * 0.05)(D, F)),
            "w_up": _w((lambda *s: _rng.normal(s) * 0.05)(D, F)),
            "w_down": _w((lambda *s: _rng.normal(s) * 0.05)(F, D)),
        }
    _B_in = _B_setup()

    return {
        "A_x": _A_in["x"],
        "A_wqkv": _A_in["wqkv"],
        "A_wo": _A_in["wo"],
        "B_x": _B_in["x"],
        "B_w_r": _B_in["w_r"],
        "B_w_gate": _B_in["w_gate"],
        "B_w_up": _B_in["w_up"],
        "B_w_down": _B_in["w_down"],
    }

def reference(A_x, A_wqkv, A_wo, B_x, B_w_r, B_w_gate, B_w_up, B_w_down):
    def _A_ref(x, wqkv, wo):
        B, S, D = x.shape
        H = 32; Dh = D // H; W = 256
        qkv = (lambda x, *d: x.transpose(*d))((x @ wqkv).reshape(B, S, 3, H, Dh), 2, 0, 3, 1, 4)
        q, k, v = qkv[0], qkv[1], qkv[2]
        scores = jnp.einsum("bhqd,bhkd->bhqk", q, k) * (Dh ** -0.5)
        idx = jnp.arange(S)
        mask = (idx[:, None] - idx[None, :] >= 0) & (idx[:, None] - idx[None, :] < W)
        scores = jnp.where(mask[None, None], scores, -1e9)
        p = _softmax(scores, axis=-1)
        o = jnp.einsum("bhqk,bhkd->bhqd", p, v)
        return (lambda x, *d: x.transpose(*d))(o, 0, 2, 1, 3).reshape(B, S, D) @ wo

    def _B_ref(x, w_r, w_gate, w_up, w_down):
        B, S, D = x.shape
        C = 1
        r = x @ w_r
        idx = jnp.argsort(-r, axis=-1)[:, :C]
        idx_e = jnp.repeat(idx.reshape(B, C, 1), D, axis=2)
        x_sel = jnp.take_along_axis(x, idx_e, axis=1)
        g = _silu(x_sel @ w_gate)
        u = x_sel @ w_up
        y = (g * u) @ w_down
        r_sel = _sigmoid(jnp.take_along_axis(r, idx, axis=1))
        y = y * r_sel.reshape(B, C, 1)
        b_off = (jnp.arange(B) * S).reshape(B, 1)
        flat_idx = (idx + b_off).reshape(B * C)
        zero = (x * 0.0).reshape(B * S, D)
        upd = _scatter_add(zero, flat_idx, y.reshape(B * C, D), axis=0)
        return x + upd.reshape(B, S, D)

    x = A_x
    x = x + _A_ref(_layernorm(x, axis=-1), A_wqkv, A_wo)
    x = x + _B_ref(_layernorm(x, axis=-1), B_w_r, B_w_gate, B_w_up, B_w_down)
    x = x + _A_ref(_layernorm(x, axis=-1), A_wqkv, A_wo)
    x = x + _B_ref(_layernorm(x, axis=-1), B_w_r, B_w_gate, B_w_up, B_w_down)
    return x
```

```python
import jax
import jax.numpy as jnp
from jax import lax
import jax.experimental.pallas as pl
import jax.experimental.pallas.tpu as pltpu

F32 = jnp.float32
BF16 = jnp.bfloat16
I32 = jnp.int32

S, D, F = 2048, 1024, 3584
TB = 256
NB = S // TB
G = D // 128
SCALE = 0.1767578125
LOG2E = 1.4426950408889634
EPS = 1.0013580322265625e-05
NT = (((1,), (1,)), ((), ()))


def _rb(x):
    return x.astype(BF16).astype(F32)


def _ld(ref, lead, start, size):
    words = ref.bitcast(I32)[lead, pl.ds(start // 2, size // 2), :]
    return words


def _bf(words):
    return pltpu.bitcast(words, BF16)


def _seg(rows):
    return lax.broadcasted_iota(I32, (rows, 128), 1) >> 5


def _layernorm(x):
    m = jnp.sum(x, axis=-1, keepdims=True) * (1.0 / D)
    c = x - m
    v = jnp.sum(c * c, axis=-1, keepdims=True) * (1.0 / D)
    den = _rb(jnp.sqrt(_rb(_rb(v) + EPS)))
    return _rb(x - _rb(m)) * (1.0 / den)


def _butterfly(tiles, starts):
    def comb(a, sa, b, sb, bit, want):
        ea, eb = sa + a.shape[0], sb + b.shape[0]
        cuts = sorted({sa, ea, sb, eb})
        parts = []
        for lo, hi in zip(cuts[:-1], cuts[1:]):
            take_a = ((_seg(hi - lo) >> bit) & 1) == want
            xa = a[lo - sa:hi - sa] if sa <= lo and hi <= ea else 0
            xb = b[lo - sb:hi - sb] if sb <= lo and hi <= eb else 0
            parts.append(jnp.where(take_a, xa, xb))
        return (jnp.concatenate(parts, axis=0) if len(parts) > 1 else parts[0]), cuts[0]

    st = {}
    for j1 in range(2):
        for h0 in range(2):
            st[j1, h0] = comb(tiles[2 * j1], starts[2 * j1], tiles[2 * j1 + 1], starts[2 * j1 + 1], 0, h0)
    return [comb(*st[0, h & 1], *st[1, h & 1], 1, h >> 1)[0] for h in range(4)]


def _kernel(x_hbm, wqkv_hbm, wo_hbm, wr_ref, wg_hbm, wu_hbm, wd_hbm, out_hbm,
            x_s, x1_s, xn_s, q_s, k_s, vt_s, o_s, p_s, wqkv_s, wvt_s, wo_s, wg_s, wu_s, wd_s,
            best_s, bidx_s, sem_x, sem_w, sem_f, sem_o):

    def rows(blk, off=0, size=TB):
        return pl.ds(pl.multiple_of(blk * TB + off, 16), size)

    x_cp = [pltpu.make_async_copy(x_hbm.at[pl.ds(0, TB)], x_s.at[pl.ds(0, TB)], sem_x.at[0]),
            pltpu.make_async_copy(x_hbm.at[pl.ds(TB, S - TB)], x_s.at[pl.ds(TB, S - TB)], sem_x.at[1])]
    wqkv_cp = pltpu.make_async_copy(wqkv_hbm, wqkv_s, sem_w.at[0])
    wo_cp = pltpu.make_async_copy(wo_hbm, wo_s, sem_w.at[1])
    ffn_cp = [pltpu.make_async_copy(wg_hbm, wg_s, sem_f.at[0]),
              pltpu.make_async_copy(wu_hbm, wu_s, sem_f.at[1]),
              pltpu.make_async_copy(wd_hbm, wd_s, sem_f.at[2])]

    def out_cp(blk):
        return pltpu.make_async_copy(x_s.at[rows(blk)], out_hbm.at[rows(blk)], sem_o.at[0])

    x_cp[0].start()
    wqkv_cp.start()
    x_cp[1].start()
    wo_cp.start()

    r32 = lax.broadcasted_iota(I32, (32, 128), 0)
    first = r32 > (lax.broadcasted_iota(I32, (32, 128), 1) & 31)
    r16 = lax.broadcasted_iota(I32, (16, 128), 0)
    t16 = lax.broadcasted_iota(I32, (16, 128), 1) & 31
    first_w = jnp.where(2 * r16 > t16, 0xFFFF, 0) | jnp.where(2 * r16 + 1 > t16, -65536, 0)

    def ln_in(blk, off, size):
        xn = _layernorm(x_s[rows(blk, off, size), :].astype(F32)).astype(BF16)
        for g in range(G):
            xn_s[g, rows(blk, off, size), :] = xn[:, g * 128:(g + 1) * 128]

    def proj(blk, g):
        xn = _bf(jnp.concatenate([_ld(xn_s, t, blk * TB, TB) for t in range(G)], axis=1))
        cols = slice(g * 128, (g + 1) * 128)
        q_s[g, rows(blk), :] = jnp.dot(xn, wqkv_s[:, cols], preferred_element_type=F32).astype(BF16)
        cols = slice(D + g * 128, D + (g + 1) * 128)
        k_s[g, rows(blk), :] = jnp.dot(xn, wqkv_s[:, cols], preferred_element_type=F32).astype(BF16)
        wvt = _bf(jnp.concatenate([_ld(wvt_s, t, g * 128, 128) for t in range(G)], axis=1))
        vt = lax.dot_general(wvt, xn, NT, preferred_element_type=F32)
        for t in range(TB // 128):
            vt_s[blk * (TB // 128) + t, pl.ds(g * 128, 128), :] = vt[:, t * 128:(t + 1) * 128].astype(BF16)

    def qk(i, g, j, nprev):
        q = _ld(q_s, g, i * 128 + 32 * j, 32)
        w = jnp.concatenate([jnp.where(_seg(16) == (s ^ j), q, 0) for s in range(4)], axis=0)
        if nprev == 2:
            k = _ld(k_s, g, i * 128 + 32 * j - 256, 288)
        else:
            k = _ld(k_s, g, 0, nprev * 128 + 32 * j + 32)
        return lax.dot_general(_bf(k), _bf(w), NT, preferred_element_type=F32)

    def softmax(s, nprev, slot):
        n = s.shape[0]
        if nprev == 2:
            sm = jnp.concatenate([jnp.where(first, s[0:32], s[256:288]), s[32:256]], axis=0)
        else:
            sm = jnp.where(first, -jnp.inf, s[n - 32:n])
            if n > 32:
                sm = jnp.concatenate([sm, s[0:n - 32]], axis=0)
        mx = jnp.max(sm, axis=0, keepdims=True)
        p = jnp.exp2((sm - mx) * (SCALE * LOG2E))
        l = jnp.sum(p, axis=0, keepdims=True)
        m = p.shape[0]
        p_s[slot, pl.ds(0, m), :] = p.astype(BF16)
        pw = _ld(p_s, slot, 0, m)
        if nprev == 2:
            old = pw[0:16] & first_w
            pw = jnp.concatenate([old, pw[16:], pw[0:16] ^ old], axis=0)
        elif n > 32:
            pw = jnp.concatenate([pw[16:], pw[0:16]], axis=0)
        return pw, jnp.broadcast_to(1.0 / _rb(l), (8, 128))

    def pv(i, g, nprev, sm):
        p = _butterfly([a for a, _ in sm], [16 * j if nprev == 2 else 0 for j in range(4)])
        linv = _butterfly([b for _, b in sm], [0] * 4)
        outs = []
        for h in range(4):
            acc = None
            for t in range(nprev + 1):
                v = _ld(vt_s, i - nprev + t, g * 128 + 32 * h, 32)
                r = jnp.dot(_bf(v), _bf(p[h][64 * t:64 * t + 64]), preferred_element_type=F32)
                acc = r if acc is None else acc + r
            outs.append(acc * jnp.concatenate([linv[h]] * 4, axis=0))
        o = pltpu.bitcast(jnp.concatenate(outs, axis=0).astype(BF16).T, I32)
        b = [o[16 * s:16 * s + 16] for s in range(4)]
        b = [jnp.where((_seg(16) & 1) == 0, b[s], b[s ^ 1]) for s in range(4)]
        b = [jnp.where((_seg(16) & 2) == 0, b[s], b[s ^ 2]) for s in range(4)]
        o_s[g, pl.ds(pl.multiple_of(i * 64, 8), 64), :] = jnp.concatenate(b, axis=0)

    def wo_mm(blk, off, size):
        o = _bf(jnp.concatenate(
            [o_s[t, pl.ds(pl.multiple_of((blk * TB + off) // 2, 8), size // 2), :] for t in range(G)], axis=1))
        a = jnp.dot(o, wo_s[...], preferred_element_type=F32)
        x1_s[rows(blk, off, size), :] = (x_s[rows(blk, off, size), :].astype(F32) + _rb(a)).astype(BF16)

    def epilogue(blk, off, size, valid=None):
        x1 = x1_s[rows(blk, off, size), :].astype(F32)
        xn = _rb(_layernorm(x1))
        x_s[rows(blk, off, size), :] = (x1 + xn).astype(BF16)
        r = _rb(jnp.sum(xn * wr_ref[...].astype(F32), axis=-1, keepdims=True))
        if valid is not None:
            r = jnp.where(valid, r, -jnp.inf)
        best, bidx = best_s[...], bidx_s[...]
        tok = lax.broadcasted_iota(I32, (8, 128), 0) + (blk * TB + off)
        for t in range(size // 8):
            rt = jnp.broadcast_to(r[8 * t:8 * t + 8], (8, 128))
            up = rt > best
            best = jnp.where(up, rt, best)
            bidx = jnp.where(up, tok + 8 * t, bidx)
        best_s[...] = best
        bidx_s[...] = bidx

    def body(b, head):
        nq = TB // 128
        units = [(g, a) for g in range(G) for a in range(nq)]
        nprev = [min(a, 2) if head else 2 for a in range(nq)]
        nxt = 1 if head else lax.rem(b + 1, NB)
        proj(b, 0)
        if not head:
            eb = jnp.where(b >= 2, b - 2, NB)
            for c in range(TB // 64):
                epilogue(eb, 64 * c, 64, valid=b >= 2)
        sc, sm = {}, {}
        for u in range(len(units) + 2):
            if u < len(units):
                g, a = units[u]
                sc[u] = [qk(b * nq + a, g, j, nprev[a]) for j in range(4)]
            if 0 <= u - 2:
                g, a = units[u - 2]
                pv(b * nq + a, g, nprev[a], sm.pop(u - 2))
            if u % nq == 0 and u // nq + 1 < G:
                proj(b, u // nq + 1)
            if u == len(units) - 1 and not head:
                wo_mm(b - 1, 0, TB // 2)
            if u == len(units) and not head:
                wo_mm(b - 1, TB // 2, TB // 2)
            if 0 <= u - 1 < len(units):
                g, a = units[u - 1]
                sm[u - 1] = [softmax(s, nprev[a], ((u - 1) % 2) * 4 + j) for j, s in enumerate(sc.pop(u - 1))]
            if u % 4 == 1 and u // 4 < TB // 64:
                ln_in(nxt, 64 * (u // 4), 64)

    def routed_token():
        best, bidx = best_s[...], bidx_s[...]
        top = jnp.max(best, axis=0, keepdims=True)
        idx = jnp.min(jnp.where(best == top, bidx, S - 1))
        grp = pl.multiple_of((idx >> 4) << 4, 16)
        x1 = x1_s[pl.ds(grp, 16), :].astype(F32)
        xn = _layernorm(x1).astype(BF16)
        gate = _rb(jnp.dot(xn, wg_s[...], preferred_element_type=F32))
        up = _rb(jnp.dot(xn, wu_s[...], preferred_element_type=F32))
        hid = (_rb(gate * jax.nn.sigmoid(gate)) * up).astype(BF16)
        y = _rb(jnp.dot(hid, wd_s[...], preferred_element_type=F32))
        y = _rb(y * _rb(jax.nn.sigmoid(top[:, 0:1])))
        xn = xn.astype(F32)
        sel = lax.broadcasted_iota(I32, (16, D), 0) == (idx & 15)
        x2 = (x1 + jnp.where(sel, _rb(xn + y), xn)).astype(BF16)
        return grp, x2

    x1_s[rows(NB), :] = jnp.zeros((TB, D), BF16)
    x_cp[0].wait()
    for c in range(TB // 64):
        ln_in(0, 64 * c, 64)
    wqkv_cp.wait()
    for t in range(G):
        for g in range(G):
            wvt_s[t, pl.ds(g * 128, 128), :] = wqkv_s[t * 128:(t + 1) * 128, 2 * D + g * 128:2 * D + (g + 1) * 128].T
    x_cp[1].wait()
    wo_cp.wait()
    for cp in ffn_cp:
        cp.start()

    def layer(li, carry):
        best_s[...] = jnp.full((8, 128), -jnp.inf, F32)
        bidx_s[...] = jnp.zeros((8, 128), I32)
        body(0, True)

        def step(b, c):
            body(b, False)

            @pl.when(jnp.logical_and(li == 1, b >= 2))
            def _():
                out_cp(b - 2).start()
            return c

        lax.fori_loop(1, NB, step, 0)
        for c in range(TB // 64):
            wo_mm(NB - 1, 64 * c, 64)
            epilogue(NB - 2, 64 * c, 64)
        for c in range(TB // 64):
            epilogue(NB - 1, 64 * c, 64)

        @pl.when(li == 0)
        def _():
            for cp in ffn_cp:
                cp.wait()

        @pl.when(li == 1)
        def _():
            out_cp(NB - 2).start()
            out_cp(NB - 1).start()

        grp, x2 = routed_token()

        @pl.when(li == 0)
        def _():
            x_s[pl.ds(grp, 16), :] = x2
            xn = _layernorm(x2.astype(F32)).astype(BF16)
            for g in range(G):
                xn_s[g, pl.ds(grp, 16), :] = xn[:, g * 128:(g + 1) * 128]

        @pl.when(li == 1)
        def _():
            for blk in range(NB):
                out_cp(blk).wait()
            x_s[pl.ds(grp, 16), :] = x2
            cp = pltpu.make_async_copy(x_s.at[pl.ds(grp, 16)], out_hbm.at[pl.ds(grp, 16)], sem_o.at[0])
            cp.start()
            cp.wait()

        return carry

    lax.fori_loop(0, 2, layer, 0)


@jax.jit
def pallas_interleave_layers__sliding_block__moe_arch_mod__prompt_kernel(
    A_x: jax.Array,
    A_wqkv: jax.Array,
    A_wo: jax.Array,
    B_x: jax.Array,
    B_w_r: jax.Array,
    B_w_gate: jax.Array,
    B_w_up: jax.Array,
    B_w_down: jax.Array,
):
    del B_x
    hbm = pl.BlockSpec(memory_space=pl.ANY)
    out = pl.pallas_call(
        _kernel,
        out_shape=jax.ShapeDtypeStruct((S, D), BF16),
        in_specs=[hbm, hbm, hbm, pl.BlockSpec(memory_space=pltpu.VMEM), hbm, hbm, hbm],
        out_specs=hbm,
        scratch_shapes=[
            pltpu.VMEM((S + TB, D), BF16),
            pltpu.VMEM((S + TB, D), BF16),
            pltpu.VMEM((G, S, 128), BF16),
            pltpu.VMEM((G, S, 128), BF16),
            pltpu.VMEM((G, S, 128), BF16),
            pltpu.VMEM((S // 128, D, 128), BF16),
            pltpu.VMEM((G, S // 2, 128), I32),
            pltpu.VMEM((8, 256, 128), BF16),
            pltpu.VMEM((D, 3 * D), BF16),
            pltpu.VMEM((G, D, 128), BF16),
            pltpu.VMEM((D, D), BF16),
            pltpu.VMEM((D, F), BF16),
            pltpu.VMEM((D, F), BF16),
            pltpu.VMEM((F, D), BF16),
            pltpu.VMEM((8, 128), F32),
            pltpu.VMEM((8, 128), I32),
            pltpu.SemaphoreType.DMA((2,)),
            pltpu.SemaphoreType.DMA((2,)),
            pltpu.SemaphoreType.DMA((3,)),
            pltpu.SemaphoreType.DMA((1,)),
        ],
        compiler_params=pltpu.CompilerParams(vmem_limit_bytes=100 * 1024 * 1024),
    )(A_x.reshape(S, D), A_wqkv, A_wo, B_w_r.reshape(1, D), B_w_gate, B_w_up, B_w_down)
    return out.reshape(1, S, D)
```

```python
import jax
import jax.numpy as jnp
from jax import lax
import jax.experimental.pallas as pl
import jax.experimental.pallas.tpu as pltpu

F32 = jnp.float32
BF16 = jnp.bfloat16
I32 = jnp.int32

S, D, F = 2048, 1024, 3584
TB = 256
NB = S // TB
MC = 128
AHEAD = 7
WAITS = (0, 1, 2, 4, 6, 8)
LAG = 5
PV = (0, 2, 4, 5)
FILL = ((1, 5), (1, 5), (1,))
LEAD = 12
G = D // 128
SCALE = 0.1767578125
LOG2E = 1.4426950408889634
EPS = 1.0013580322265625e-05
NT = (((1,), (1,)), ((), ()))


def _rb(x):
    return x.astype(BF16).astype(F32)


def _ld(ref, lead, start, size):
    return ref[lead].bitcast(I32)[pl.ds(start // 2, size // 2), :]


def _bf(words):
    return pltpu.bitcast(words, BF16)


def _seg(rows):
    return lax.broadcasted_iota(I32, (rows, 128), 1) >> 5


def _layernorm(x):
    m = jnp.sum(x, axis=-1, keepdims=True) * (1.0 / D)
    c = x - m
    v = jnp.sum(c * c, axis=-1, keepdims=True) * (1.0 / D)
    den = _rb(jnp.sqrt(_rb(_rb(v) + EPS)))
    return _rb(x - _rb(m)) * (1.0 / den)


def _butterfly(tiles, starts):
    def comb(a, sa, b, sb, bit, want):
        ea, eb = sa + a.shape[0], sb + b.shape[0]
        cuts = sorted({sa, ea, sb, eb})
        parts = []
        for lo, hi in zip(cuts[:-1], cuts[1:]):
            take_a = ((_seg(hi - lo) >> bit) & 1) == want
            xa = a[lo - sa:hi - sa] if sa <= lo and hi <= ea else 0
            xb = b[lo - sb:hi - sb] if sb <= lo and hi <= eb else 0
            parts.append(jnp.where(take_a, xa, xb))
        return (jnp.concatenate(parts, axis=0) if len(parts) > 1 else parts[0]), cuts[0]

    st = {}
    for j1 in range(2):
        for h0 in range(2):
            st[j1, h0] = comb(tiles[2 * j1], starts[2 * j1], tiles[2 * j1 + 1], starts[2 * j1 + 1], 0, h0)
    return [comb(*st[0, h & 1], *st[1, h & 1], 1, h >> 1)[0] for h in range(4)]


def _kernel(x_hbm, wqkv_hbm, wo_hbm, wr_ref, wg_hbm, wu_hbm, wd_hbm, out_hbm,
            x_s, x1_s, xn_s, q_s, k_s, vt_s, o_s, p_s, wqkv_s, wvt_s, wo_s, wg_s, wu_s, wd_s,
            best_s, bidx_s, zero_s, sem_x, sem_w, sem_f, sem_o):

    def rows(blk, off=0, size=TB):
        return pl.ds(pl.multiple_of(blk * TB + off, 16), size)

    x_cp = [pltpu.make_async_copy(x_hbm.at[pl.ds(lo, n)], x_s.at[pl.ds(lo, n)], sem_x.at[i])
            for i, (lo, n) in enumerate(((0, 128), (128, TB - 128), (TB, TB), (2 * TB, 2 * TB), (4 * TB, S - 4 * TB)))]
    w_cp = [pltpu.make_async_copy(wqkv_hbm.at[:, pl.ds(c * 128, 128)], wqkv_s[c], sem_w.at[c])
            for c in range(3 * G)]
    wo_cp = [pltpu.make_async_copy(wo_hbm.at[:, pl.ds(c * 128, 128)], wo_s[c], sem_w.at[3 * G + c])
             for c in range(G)]
    ffn_cp = [pltpu.make_async_copy(src.at[:, pl.ds(c * 128, 128)], dst.at[c], sem_f.at[0])
              for src, dst in ((wg_hbm, wg_s), (wu_hbm, wu_s), (wd_hbm, wd_s)) for c in range(dst.shape[0])]

    def out_cp(blk):
        return pltpu.make_async_copy(x_s.at[rows(blk)], out_hbm.at[rows(blk)], sem_o.at[0])

    queue = [x_cp[0], w_cp[2 * G], x_cp[1]]
    for g in range(G):
        queue += [w_cp[G + g], w_cp[g]] + w_cp[2 * G + g + 1:2 * G + g + 2] + ([x_cp[2]] if g == 1 else [])
    queue += wo_cp + [x_cp[3]]
    flight = dict(started=0, waited=0)

    def arrive(cp):
        n = next(i for i, c in enumerate(queue) if c is cp) + 1
        while flight["waited"] < n:
            while flight["started"] < min(flight["waited"] + AHEAD, len(queue)):
                queue[flight["started"]].start()
                flight["started"] += 1
            queue[flight["waited"]].wait()
            flight["waited"] += 1
        while flight["started"] < min(flight["waited"] + AHEAD, len(queue)):
            queue[flight["started"]].start()
            flight["started"] += 1

    def transpose_wv(g):
        for c in range(G):
            wvt_s[c][pl.ds(g * 128, 128), :] = wqkv_s[2 * G + g][pl.ds(c * 128, 128), :].T

    r32 = lax.broadcasted_iota(I32, (32, 128), 0)
    first = r32 > (lax.broadcasted_iota(I32, (32, 128), 1) & 31)
    r16 = lax.broadcasted_iota(I32, (16, 128), 0)
    t16 = lax.broadcasted_iota(I32, (16, 128), 1) & 31
    first_w = jnp.where(2 * r16 > t16, 0xFFFF, 0) | jnp.where(2 * r16 + 1 > t16, -65536, 0)

    def after(x, tok):
        if tok is None:
            return x
        never, val = tok
        reps = (x.shape[0] // 8, x.shape[1] // 128)
        val = lax.bitcast_convert_type(val, x.dtype)
        return jnp.where(jnp.tile(never, reps) < 0, jnp.tile(val, reps), x)

    def words_after(w, tok):
        if tok is None:
            return w
        return jnp.concatenate([after(w[0:8], tok), w[8:]], axis=0)

    def ln_in(blk, off, size, tok=None):
        xf = _layernorm(after(x_s[rows(blk, off, size), :].astype(F32), tok))
        xn = xf.astype(BF16)

        def store():
            for g in range(G):
                xn_s[g][rows(blk, off, size), :] = xn[:, g * 128:(g + 1) * 128]

        return xf[size - 8:, D - 128:], store

    def xn_rows(blk, off, size, tok=None):
        return _bf(join([_ld(xn_s, t, blk * TB + off, size) for t in range(G)], tok))

    def join(slabs, tok):
        return jnp.concatenate([words_after(w, tok if t < 4 else None) for t, w in enumerate(slabs)], axis=1)

    def proj_qk(blk, g, which, off, size, tok):
        w = _bf(_ld(wqkv_s, which * G + g, 0, D))
        y = jnp.dot(xn_rows(blk, off, size, tok), w, preferred_element_type=F32)
        (q_s, k_s)[which][g][rows(blk, off, size), :] = y.astype(BF16)
        return y

    def proj_v(blk, g, t, tok):
        wvt = _bf(join([_ld(wvt_s, c, g * 128, 128) for c in range(G)], tok))
        vt = lax.dot_general(wvt, xn_rows(blk, 128 * t, 128), NT, preferred_element_type=F32)
        vt_s[g][rows(blk, 128 * t, 128), :] = vt.astype(BF16)
        return vt

    def qk(i, g, j, nprev):
        q = _ld(q_s, g, i * 128 + 32 * j, 32)
        w = jnp.concatenate([jnp.where(_seg(16) == (s ^ j), q, 0) for s in range(4)], axis=0)
        if nprev == 2:
            k = _ld(k_s, g, i * 128 + 32 * j - 256, 288)
        else:
            k = _ld(k_s, g, 0, nprev * 128 + 32 * j + 32)
        return lax.dot_general(_bf(k), _bf(w), NT, preferred_element_type=F32)

    def softmax(s, nprev, slot, tok):
        n = s.shape[0]
        if nprev == 2:
            sm = jnp.concatenate([jnp.where(first, s[0:32], s[256:288]), s[32:256]], axis=0)
        else:
            sm = jnp.where(first, -jnp.inf, s[n - 32:n])
            if n > 32:
                sm = jnp.concatenate([sm, s[0:n - 32]], axis=0)
        mx = after(jnp.broadcast_to(jnp.max(sm, axis=0, keepdims=True), (8, 128)), tok)
        mx = jnp.tile(mx, (sm.shape[0] // 8, 1))
        p = jnp.exp2((sm - mx) * (SCALE * LOG2E))
        l = jnp.sum(p, axis=0, keepdims=True)
        m = p.shape[0]
        p_s[slot][pl.ds(0, m), :] = p.astype(BF16)
        return jnp.broadcast_to(1.0 / _rb(l), (8, 128))

    def p_words(slot, j, nprev, lo, hi):
        n = 144 if nprev == 2 else nprev * 64 + 16 * j + 16
        parts = []
        for r in range(lo, hi, 16):
            if r == n - 16:
                w = _ld(p_s, slot, 0, 32)
                parts.append(w & ~first_w if nprev == 2 else w)
            elif nprev == 2:
                w = _ld(p_s, slot, 2 * r, 32)
                parts.append(w & first_w if r == 0 else w)
            else:
                parts.append(_ld(p_s, slot, 2 * r + 32, 32))
        return jnp.concatenate(parts, axis=0) if len(parts) > 1 else parts[0]

    def pv(i, g, nprev, slot, t, acc):
        tiles, starts = [], []
        for j in range(4):
            st = 16 * j if nprev == 2 else 0
            n = 144 if nprev == 2 else nprev * 64 + 16 * j + 16
            lo, hi = max(64 * t, st), min(64 * t + 64, st + n)
            tiles.append(p_words(slot + j, j, nprev, lo - st, hi - st))
            starts.append(lo)
        p = _butterfly(tiles, starts)
        out = []
        for h in range(4):
            v = _ld(vt_s, g, (i - nprev + t) * 128 + 32 * h, 32)
            r = jnp.dot(_bf(v), _bf(p[h]), preferred_element_type=F32)
            out.append(r if acc is None else acc[h] + r)
        return out

    def att_out(i, g, acc, linv):
        linv = _butterfly(linv, [0] * 4)
        o = jnp.concatenate([acc[h] * jnp.concatenate([linv[h]] * 4, axis=0) for h in range(4)], axis=0)
        o = pltpu.bitcast(o.astype(BF16).T, I32)
        b = [o[16 * s:16 * s + 16] for s in range(4)]
        b = [jnp.where((_seg(16) & 1) == 0, b[s], b[s ^ 1]) for s in range(4)]
        b = [jnp.where((_seg(16) & 2) == 0, b[s], b[s ^ 2]) for s in range(4)]

        def store():
            o_s[g][pl.ds(pl.multiple_of(i * 64, 8), 64), :] = jnp.concatenate(b, axis=0)

        return store

    def wo_mm(blk, off, size, c0=0, cn=D, tok=None):
        o = _bf(join(
            [o_s[t][pl.ds(pl.multiple_of((blk * TB + off) // 2, 8), size // 2), :] for t in range(G)], tok))
        a = jnp.dot(o, _bf(jnp.concatenate([_ld(wo_s, c, 0, D) for c in range(c0 // 128, (c0 + cn) // 128)], axis=1)), preferred_element_type=F32)
        x = x_s[rows(blk, off, size), c0:c0 + cn].astype(F32)
        x1_s[rows(blk, off, size), c0:c0 + cn] = (x + _rb(a)).astype(BF16)
        return a[:, 0:128]

    def epilogue(blk, off, size, valid=None, tok=None):
        x1 = after(x1_s[rows(blk, off, size), :].astype(F32), tok)
        xn = _rb(_layernorm(x1))
        x2 = (x1 + xn).astype(BF16)
        r = _rb(jnp.sum(xn * wr_ref[...].astype(F32).reshape(1, D), axis=-1, keepdims=True))
        if valid is not None:
            r = jnp.where(valid, r, -jnp.inf)
        best, bidx = best_s[...], bidx_s[...]
        pos = lax.broadcasted_iota(I32, (8, 128), 0) + (blk * TB + off)
        for t in range(size // 8):
            rt = jnp.broadcast_to(r[8 * t:8 * t + 8], (8, 128))
            up = rt > best
            best = jnp.where(up, rt, best)
            bidx = jnp.where(up, pos + 8 * t, bidx)
        best_s[...] = best
        bidx_s[...] = bidx

        def store():
            x_s[rows(blk, off, size), :] = x2

        return best, store

    def body(b, head, cold=False):
        nq = TB // 128
        units = [(g, a) for g in range(G) for a in range(nq)]
        nprev = [min(a, 2) if head else 2 for a in range(nq)]
        nxt = 1 if head else lax.rem(b + 1, NB)

        def qk_task(tk, g, w, o):
            if cold and o == 0 and w == 1 and g in WAITS:
                upto = WAITS[WAITS.index(g) + 1]
                arrive(w_cp[2 * G + upto] if upto < G else w_cp[G - 1])
            return proj_qk(b, g, w, o, MC, tk)

        def v_task(tk, g, t):
            y = proj_v(b, g, t, tk)
            if cold and t == 0 and g + 1 < G:
                transpose_wv(g + 1)
            return y

        def ln_task(tk, o):
            if cold and o == 0:
                arrive(x_cp[2])
            return ln_in(nxt, o, 16, tk)

        mm = []
        for g in range(G):
            for t in range(nq):
                for which in (1, 0):
                    for off in range(0, 128, MC):
                        mm.append(lambda tk, g=g, w=which, o=128 * t + off: qk_task(tk, g, w, o))
                        mm.extend([None] * (MC // 64 - 1))
                mm.extend([lambda tk, g=g, t=t: v_task(tk, g, t), None])
        if not head:
            for off in range(0, TB, MC):
                for c in range(G):
                    mm.append(lambda tk, o=off, c=c: wo_mm(b - 1, o, MC, 128 * c, 128, tk))
                    mm.extend([None] * (MC // 64 - 1))
        rowwise = [lambda tk, o=o: ln_task(tk, o) for o in range(0, TB, 16)]
        if not head:
            eb = jnp.where(b >= 2, b - 2, NB)
            rowwise = [lambda tk, o=o: epilogue(eb, o, 16, b >= 2, tk) for o in range(0, TB, 16)] + rowwise

        never = zero_s[...]
        st = dict(slot=0, y=None, tok=None, due=[])

        def dense():
            if not mm:
                st["tok"] = None
                return
            f = mm.pop(0)
            st["slot"] += 1
            st["tok"] = None if st["y"] is None else (never, st["y"][0:8])
            if f is None:
                st["y"] = st["y"][st["y"].shape[0] - 8:]
                return
            due = None
            while st["due"] and st["due"][0][0] <= st["slot"]:
                v, store = st["due"].pop(0)[1]
                store()
                due = (never, after(v, due))
            st["y"] = f(due)

        def fill():
            if rowwise:
                st["due"].append((st["slot"] + LAG, rowwise.pop(0)(st["tok"])))

        for c in range(LEAD):
            dense()
            if c % 2 == 1 and not head:
                fill()
        late = []
        sc, linv = {}, {}
        for u in range(len(units) + 1):
            if u < len(units):
                g, a = units[u]
                sc[u] = [qk(b * nq + a, g, j, nprev[a]) for j in range(4)]
                linv[u] = []
            acc = None
            for c in range(6):
                dense()
                if u >= 1:
                    pg, pa = units[u - 1]
                    if c in PV[:nprev[pa] + 1]:
                        acc = pv(b * nq + pa, pg, nprev[pa], ((u - 1) % 2) * 4, PV.index(c), acc)
                    if c == PV[3]:
                        store = att_out(b * nq + pa, pg, acc, linv.pop(u - 1))
                        if pg == G - 1:
                            late.append(store)
                        else:
                            store()
                if u < len(units) and c >= 2:
                    linv[u].append(softmax(sc[u][c - 2], nprev[a], (u % 2) * 4 + c - 2, st["tok"]))
                if c in FILL[u % len(FILL)] and (u >= 2 or not head):
                    fill()
        while mm or rowwise:
            dense()
            dense()
            fill()
        for _, (_, store) in st["due"]:
            store()
        for store in late:
            store()

    def tail():
        never = zero_s[...]
        rowwise = [(NB - 2, o) for o in range(0, TB, 16)]
        y, due, n = None, [], 0
        for off in range(0, TB, 64):
            for c0 in range(0, D, 256):
                tok = None if y is None else (never, y[0:8])
                wait = None
                while due and due[0][0] <= n:
                    v, store = due.pop(0)[1]
                    store()
                    wait = (never, after(v, wait))
                y = wo_mm(NB - 1, off, 64, c0, 256, wait)
                for _ in range(2):
                    if rowwise:
                        due.append((n + 3, epilogue(*rowwise.pop(0), 16, None, tok)))
                n += 1
            rowwise += [(NB - 1, off + o) for o in range(0, 64, 16)]
        due += [(0, epilogue(*r, 16)) for r in rowwise]
        for _, (_, store) in due:
            store()

    def routed_token():
        best, bidx = best_s[...], bidx_s[...]
        top = jnp.max(best, axis=0, keepdims=True)
        idx = jnp.min(jnp.where(best == top, bidx, S - 1))
        grp = pl.multiple_of((idx >> 4) << 4, 16)
        x1 = x1_s[pl.ds(grp, 16), :].astype(F32)
        xn = _layernorm(x1).astype(BF16)
        nf = F // 128 // 2

        def half(i, y):
            def cols(w_s):
                return _bf(jnp.concatenate([w_s.bitcast(I32)[i * nf + c] for c in range(nf)], axis=1))

            hid = []
            for c in range(0, nf * 128, 256):
                gate = _rb(jnp.dot(xn, cols(wg_s)[:, c:c + 256], preferred_element_type=F32))
                up = _rb(jnp.dot(xn, cols(wu_s)[:, c:c + 256], preferred_element_type=F32))
                hid.append((_rb(gate * jax.nn.sigmoid(gate)) * up).astype(BF16))
            for c, h in enumerate(hid):
                r = pl.ds(pl.multiple_of(i * (nf * 64) + c * 128, 8), 128)
                wd = jnp.concatenate([wd_s.bitcast(I32)[n, r, :] for n in range(G)], axis=1)
                y = y + jnp.dot(h, _bf(wd), preferred_element_type=F32)
            return y

        y = _rb(lax.fori_loop(0, 2, half, jnp.zeros((16, D), F32)))
        y = _rb(y * _rb(jax.nn.sigmoid(top[:, 0:1])))
        xn = xn.astype(F32)
        sel = lax.broadcasted_iota(I32, (16, D), 0) == (idx & 15)
        x2 = (x1 + jnp.where(sel, _rb(xn + y), xn)).astype(BF16)
        return grp, x2

    zero_s[...] = jnp.zeros((8, 128), I32)
    x1_s[rows(NB), :] = jnp.zeros((TB, D), BF16)
    for c in range(TB // 64):
        arrive(x_cp[c // 2])
        ln_in(0, 64 * c, 64)[1]()
    transpose_wv(0)
    body(0, True, cold=True)
    arrive(queue[-1])

    def layer(li, carry):
        best_s[...] = jnp.full((8, 128), -jnp.inf, F32)
        bidx_s[...] = jnp.zeros((8, 128), I32)

        def step(b, c):
            body(b, False)

            @pl.when(jnp.logical_and(li == 0, b == 1))
            def _():
                x_cp[4].start()

            @pl.when(jnp.logical_and(li == 0, b == 2))
            def _():
                x_cp[4].wait()
                for cp in ffn_cp:
                    cp.start()

            @pl.when(jnp.logical_and(li == 1, b >= 2))
            def _():
                out_cp(b - 2).start()
            return c

        lax.fori_loop(1, NB, step, 0)
        tail()

        @pl.when(li == 0)
        def _():
            for cp in ffn_cp:
                cp.wait()

        @pl.when(li == 1)
        def _():
            out_cp(NB - 2).start()
            out_cp(NB - 1).start()

        grp, x2 = routed_token()

        @pl.when(li == 0)
        def _():
            x_s[pl.ds(grp, 16), :] = x2
            xn = _layernorm(x2.astype(F32)).astype(BF16)
            for g in range(G):
                xn_s[g][pl.ds(grp, 16), :] = xn[:, g * 128:(g + 1) * 128]
            body(0, True)

        @pl.when(li == 1)
        def _():
            for blk in range(NB):
                out_cp(blk).wait()
            x_s[pl.ds(grp, 16), :] = x2
            cp = pltpu.make_async_copy(x_s.at[pl.ds(grp, 16)], out_hbm.at[pl.ds(grp, 16)], sem_o.at[0])
            cp.start()
            cp.wait()

        return carry

    lax.fori_loop(0, 2, layer, 0)


@jax.jit
def pallas_interleave_layers__sliding_block__moe_arch_mod__prompt_kernel(
    A_x: jax.Array,
    A_wqkv: jax.Array,
    A_wo: jax.Array,
    B_x: jax.Array,
    B_w_r: jax.Array,
    B_w_gate: jax.Array,
    B_w_up: jax.Array,
    B_w_down: jax.Array,
):
    del B_x
    hbm = pl.BlockSpec(memory_space=pl.ANY)
    out = pl.pallas_call(
        _kernel,
        out_shape=jax.ShapeDtypeStruct((S, D), BF16),
        in_specs=[hbm, hbm, hbm, pl.BlockSpec(memory_space=pltpu.VMEM), hbm, hbm, hbm],
        out_specs=hbm,
        scratch_shapes=[
            pltpu.VMEM((S + TB, D), BF16),
            pltpu.VMEM((S + TB, D), BF16),
            [pltpu.VMEM((S, 128), BF16)] * G,
            [pltpu.VMEM((S, 128), BF16)] * G,
            [pltpu.VMEM((S, 128), BF16)] * G,
            [pltpu.VMEM((S, 128), BF16)] * G,
            [pltpu.VMEM((S // 2, 128), I32)] * G,
            [pltpu.VMEM((256, 128), BF16)] * 8,
            [pltpu.VMEM((D, 128), BF16)] * (3 * G),
            [pltpu.VMEM((D, 128), BF16)] * G,
            [pltpu.VMEM((D, 128), BF16)] * G,
            pltpu.VMEM((F // 128, D, 128), BF16),
            pltpu.VMEM((F // 128, D, 128), BF16),
            pltpu.VMEM((G, F, 128), BF16),
            pltpu.VMEM((8, 128), F32),
            pltpu.VMEM((8, 128), I32),
            pltpu.VMEM((8, 128), I32),
            pltpu.SemaphoreType.DMA((5,)),
            pltpu.SemaphoreType.DMA((4 * G,)),
            pltpu.SemaphoreType.DMA((1,)),
            pltpu.SemaphoreType.DMA((1,)),
        ],
        compiler_params=pltpu.CompilerParams(vmem_limit_bytes=100 * 1024 * 1024),
    )(A_x.reshape(S, D), A_wqkv, A_wo, B_w_r, B_w_gate, B_w_up, B_w_down)
    return out.reshape(1, S, D)
```

```python
import jax
import jax.numpy as jnp
from jax import lax
import jax.experimental.pallas as pl
import jax.experimental.pallas.tpu as pltpu

F32 = jnp.float32
BF16 = jnp.bfloat16
I32 = jnp.int32

S, D, F = 2048, 1024, 3584
TB = 256
NB = S // TB
MC = 128
AHEAD = 7
WAITS = (0, 1, 2, 4, 6, 8)
LAG = 5
RND = 1
SM = (0, 2, 4, 5)
PV = (2, 3, 4, 5)
FILL = ((1, 5), (1,))
LEAD = 14
G = D // 128
SCALE = 0.1767578125
LOG2E = 1.4426950408889634
EPS = 1.0013580322265625e-05
NT = (((1,), (1,)), ((), ()))


def _rb(x):
    return x.astype(BF16).astype(F32)


def _ld(ref, lead, start, size):
    return ref[lead].bitcast(I32)[pl.ds(start // 2, size // 2), :]


def _bf(words):
    return pltpu.bitcast(words, BF16)


def _seg(rows):
    return lax.broadcasted_iota(I32, (rows, 128), 1) >> 5


def _layernorm(x):
    m = jnp.sum(x, axis=-1, keepdims=True) * (1.0 / D)
    c = x - m
    v = jnp.sum(c * c, axis=-1, keepdims=True) * (1.0 / D)
    den = _rb(jnp.sqrt(_rb(_rb(v) + EPS)))
    return _rb(x - _rb(m)) * (1.0 / den)


def _butterfly(tiles, starts):
    def comb(a, sa, b, sb, bit, want):
        ea, eb = sa + a.shape[0], sb + b.shape[0]
        cuts = sorted({sa, ea, sb, eb})
        parts = []
        for lo, hi in zip(cuts[:-1], cuts[1:]):
            take_a = ((_seg(hi - lo) >> bit) & 1) == want
            xa = a[lo - sa:hi - sa] if sa <= lo and hi <= ea else 0
            xb = b[lo - sb:hi - sb] if sb <= lo and hi <= eb else 0
            parts.append(jnp.where(take_a, xa, xb))
        return (jnp.concatenate(parts, axis=0) if len(parts) > 1 else parts[0]), cuts[0]

    st = {}
    for j1 in range(2):
        for h0 in range(2):
            st[j1, h0] = comb(tiles[2 * j1], starts[2 * j1], tiles[2 * j1 + 1], starts[2 * j1 + 1], 0, h0)
    return [comb(*st[0, h & 1], *st[1, h & 1], 1, h >> 1)[0] for h in range(4)]


def _kernel(x_hbm, wqkv_hbm, wo_hbm, wr_ref, wg_hbm, wu_hbm, wd_hbm, out_hbm,
            x_s, x1_s, xn_s, q_s, k_s, vt_s, o_s, s_s, p_s, wqkv_s, wvt_s, wo_s, wg_s, wu_s, wd_s,
            best_s, bidx_s, zero_s, sem_x, sem_w, sem_f, sem_o):

    def rows(blk, off=0, size=TB):
        return pl.ds(pl.multiple_of(blk * TB + off, 16), size)

    x_cp = [pltpu.make_async_copy(x_hbm.at[pl.ds(lo, n)], x_s.at[pl.ds(lo, n)], sem_x.at[i])
            for i, (lo, n) in enumerate(((0, 128), (128, TB - 128), (TB, TB), (2 * TB, 2 * TB), (4 * TB, S - 4 * TB)))]
    w_cp = [pltpu.make_async_copy(wqkv_hbm.at[:, pl.ds(c * 128, 128)], wqkv_s[c], sem_w.at[c])
            for c in range(3 * G)]
    wo_cp = [pltpu.make_async_copy(wo_hbm.at[:, pl.ds(c * 128, 128)], wo_s[c], sem_w.at[3 * G + c])
             for c in range(G)]
    ffn_cp = [pltpu.make_async_copy(src.at[:, pl.ds(c * 128, 128)], dst.at[c], sem_f.at[0])
              for src, dst in ((wg_hbm, wg_s), (wu_hbm, wu_s), (wd_hbm, wd_s)) for c in range(dst.shape[0])]

    def out_cp(blk):
        return pltpu.make_async_copy(x_s.at[rows(blk)], out_hbm.at[rows(blk)], sem_o.at[0])

    queue = [x_cp[0], w_cp[2 * G], x_cp[1]]
    for g in range(G):
        queue += [w_cp[G + g], w_cp[g]] + w_cp[2 * G + g + 1:2 * G + g + 2] + ([x_cp[2]] if g == 1 else [])
    queue += wo_cp + [x_cp[3]]
    flight = dict(started=0, waited=0)

    def arrive(cp):
        n = next(i for i, c in enumerate(queue) if c is cp) + 1
        while flight["waited"] < n:
            while flight["started"] < min(flight["waited"] + AHEAD, len(queue)):
                queue[flight["started"]].start()
                flight["started"] += 1
            queue[flight["waited"]].wait()
            flight["waited"] += 1
        while flight["started"] < min(flight["waited"] + AHEAD, len(queue)):
            queue[flight["started"]].start()
            flight["started"] += 1

    def transpose_wv(g):
        for c in range(G):
            wvt_s[c][pl.ds(g * 128, 128), :] = wqkv_s[2 * G + g][pl.ds(c * 128, 128), :].T

    r32 = lax.broadcasted_iota(I32, (32, 128), 0)
    first = r32 > (lax.broadcasted_iota(I32, (32, 128), 1) & 31)
    r16 = lax.broadcasted_iota(I32, (16, 128), 0)
    t16 = lax.broadcasted_iota(I32, (16, 128), 1) & 31
    first_w = jnp.where(2 * r16 > t16, 0xFFFF, 0) | jnp.where(2 * r16 + 1 > t16, -65536, 0)

    def after(x, tok):
        if tok is None:
            return x
        never, val = tok
        reps = (x.shape[0] // 8, x.shape[1] // 128)
        val = lax.bitcast_convert_type(val, x.dtype)
        return jnp.where(jnp.tile(never, reps) < 0, jnp.tile(val, reps), x)

    def words_after(w, tok):
        if tok is None:
            return w
        return jnp.concatenate([after(w[0:8], tok), w[8:]], axis=0)

    def ln_in(blk, off, size, tok=None):
        xf = _layernorm(after(x_s[rows(blk, off, size), :].astype(F32), tok))
        xn = xf.astype(BF16)

        def store():
            for g in range(G):
                xn_s[g][rows(blk, off, size), :] = xn[:, g * 128:(g + 1) * 128]

        return xf[size - 8:, D - 128:], store

    def xn_rows(blk, off, size, tok=None):
        return _bf(join([_ld(xn_s, t, blk * TB + off, size) for t in range(G)], tok))

    def join(slabs, tok):
        return jnp.concatenate([words_after(w, tok if t < 4 else None) for t, w in enumerate(slabs)], axis=1)

    def proj_qk(blk, g, which, off, size, tok):
        w = _bf(_ld(wqkv_s, which * G + g, 0, D))
        y = jnp.dot(xn_rows(blk, off, size, tok), w, preferred_element_type=F32)
        (q_s, k_s)[which][g][rows(blk, off, size), :] = y.astype(BF16)
        return y

    def proj_v(blk, g, t, tok):
        wvt = _bf(join([_ld(wvt_s, c, g * 128, 128) for c in range(G)], tok))
        vt = lax.dot_general(wvt, xn_rows(blk, 128 * t, 128), NT, preferred_element_type=F32)
        vt_s[g][rows(blk, 128 * t, 128), :] = vt.astype(BF16)
        return vt

    def qk(i, g, j, nprev, slot):
        q = _ld(q_s, g, i * 128 + 32 * j, 32)
        w = jnp.concatenate([jnp.where(_seg(16) == (s ^ j), q, 0) for s in range(4)], axis=0)
        if nprev == 2:
            k = _ld(k_s, g, i * 128 + 32 * j - 256, 288)
        else:
            k = _ld(k_s, g, 0, nprev * 128 + 32 * j + 32)
        s = lax.dot_general(_bf(k), _bf(w), NT, preferred_element_type=F32)
        n = s.shape[0]
        if nprev == 2:
            sm = jnp.concatenate([jnp.where(first, s[0:32], s[256:288]), s[32:256]], axis=0)
        else:
            sm = jnp.where(first, -jnp.inf, s[n - 32:n])
            if n > 32:
                sm = jnp.concatenate([sm, s[0:n - 32]], axis=0)
        mx = jnp.broadcast_to(jnp.max(sm, axis=0, keepdims=True), (8, 128))
        if RND:
            s_s[slot][pl.ds(0, sm.shape[0]), :] = sm.astype(BF16)
        return sm, mx

    def softmax(sm, mx, slot, tok):
        if RND:
            sm = _bf(_ld(s_s, slot, 0, sm.shape[0])).astype(F32)
            mx = _rb(mx)
        if RND == 2:
            scale = jnp.tile(after(jnp.full((8, 128), SCALE, F32), tok), (sm.shape[0] // 8, 1))
            sm = _rb(sm * scale)
            mx = _rb(mx * SCALE)
        mx = jnp.tile(after(mx, tok), (sm.shape[0] // 8, 1))
        p = jnp.exp2((sm - mx) * (LOG2E if RND == 2 else SCALE * LOG2E))
        l = jnp.sum(p, axis=0, keepdims=True)
        m = p.shape[0]
        p_s[slot][pl.ds(0, m), :] = p.astype(BF16)
        return jnp.broadcast_to(1.0 / _rb(l), (8, 128))

    def p_words(slot, j, nprev, lo, hi):
        n = 144 if nprev == 2 else nprev * 64 + 16 * j + 16
        parts = []
        for r in range(lo, hi, 16):
            if r == n - 16:
                w = _ld(p_s, slot, 0, 32)
                parts.append(w & ~first_w if nprev == 2 else w)
            elif nprev == 2:
                w = _ld(p_s, slot, 2 * r, 32)
                parts.append(w & first_w if r == 0 else w)
            else:
                parts.append(_ld(p_s, slot, 2 * r + 32, 32))
        return jnp.concatenate(parts, axis=0) if len(parts) > 1 else parts[0]

    def pv(i, g, nprev, slot, t, acc):
        tiles, starts = [], []
        for j in range(4):
            st = 16 * j if nprev == 2 else 0
            n = 144 if nprev == 2 else nprev * 64 + 16 * j + 16
            lo, hi = max(64 * t, st), min(64 * t + 64, st + n)
            tiles.append(p_words(slot + j, j, nprev, lo - st, hi - st))
            starts.append(lo)
        p = _butterfly(tiles, starts)
        out = []
        for h in range(4):
            v = _ld(vt_s, g, (i - nprev + t) * 128 + 32 * h, 32)
            r = jnp.dot(_bf(v), _bf(p[h]), preferred_element_type=F32)
            out.append(r if acc is None else acc[h] + r)
        return out, p[3][0:8]

    def att_out(i, g, acc, linv):
        linv = _butterfly(linv, [0] * 4)
        o = jnp.concatenate([acc[h] * jnp.concatenate([linv[h]] * 4, axis=0) for h in range(4)], axis=0)
        o = pltpu.bitcast(o.astype(BF16).T, I32)
        b = [o[16 * s:16 * s + 16] for s in range(4)]
        b = [jnp.where((_seg(16) & 1) == 0, b[s], b[s ^ 1]) for s in range(4)]
        b = [jnp.where((_seg(16) & 2) == 0, b[s], b[s ^ 2]) for s in range(4)]

        def store():
            o_s[g][pl.ds(pl.multiple_of(i * 64, 8), 64), :] = jnp.concatenate(b, axis=0)

        return store

    def wo_mm(blk, off, size, c0=0, cn=D, tok=None):
        o = _bf(join(
            [o_s[t][pl.ds(pl.multiple_of((blk * TB + off) // 2, 8), size // 2), :] for t in range(G)], tok))
        a = jnp.dot(o, _bf(jnp.concatenate([_ld(wo_s, c, 0, D) for c in range(c0 // 128, (c0 + cn) // 128)], axis=1)), preferred_element_type=F32)
        x = x_s[rows(blk, off, size), c0:c0 + cn].astype(F32)
        x1_s[rows(blk, off, size), c0:c0 + cn] = (x + _rb(a)).astype(BF16)
        return a[:, 0:128]

    def epilogue(blk, off, size, valid=None, tok=None):
        x1 = after(x1_s[rows(blk, off, size), :].astype(F32), tok)
        xn = _rb(_layernorm(x1))
        x2 = (x1 + xn).astype(BF16)
        r = _rb(jnp.sum(xn * wr_ref[...].astype(F32).reshape(1, D), axis=-1, keepdims=True))
        if valid is not None:
            r = jnp.where(valid, r, -jnp.inf)
        best, bidx = best_s[...], bidx_s[...]
        pos = lax.broadcasted_iota(I32, (8, 128), 0) + (blk * TB + off)
        for t in range(size // 8):
            rt = jnp.broadcast_to(r[8 * t:8 * t + 8], (8, 128))
            up = rt > best
            best = jnp.where(up, rt, best)
            bidx = jnp.where(up, pos + 8 * t, bidx)
        best_s[...] = best
        bidx_s[...] = bidx

        def store():
            x_s[rows(blk, off, size), :] = x2

        return best, store

    def body(b, head, cold=False):
        nq = TB // 128
        units = [(g, a) for g in range(G) for a in range(nq)]
        nprev = [min(a, 2) if head else 2 for a in range(nq)]
        nxt = 1 if head else lax.rem(b + 1, NB)

        def qk_task(tk, g, w, o):
            if cold and o == 0 and w == 1 and g in WAITS:
                upto = WAITS[WAITS.index(g) + 1]
                arrive(w_cp[2 * G + upto] if upto < G else w_cp[G - 1])
            return proj_qk(b, g, w, o, MC, tk)

        def v_task(tk, g, t):
            y = proj_v(b, g, t, tk)
            if cold and t == 0 and g + 1 < G:
                transpose_wv(g + 1)
            return y

        def ln_task(tk, o):
            if cold and o == 0:
                arrive(x_cp[2])
            return ln_in(nxt, o, 16, tk)

        mm = []
        for g in range(G):
            for t in range(nq):
                for which in (1, 0):
                    for off in range(0, 128, MC):
                        mm.append(lambda tk, g=g, w=which, o=128 * t + off: qk_task(tk, g, w, o))
                        mm.extend([None] * (MC // 64 - 1))
                mm.extend([lambda tk, g=g, t=t: v_task(tk, g, t), None])
        if not head:
            for off in range(0, TB, MC):
                for c in range(G):
                    mm.append(lambda tk, o=off, c=c: wo_mm(b - 1, o, MC, 128 * c, 128, tk))
                    mm.extend([None] * (MC // 64 - 1))
        rowwise = [lambda tk, o=o: ln_task(tk, o) for o in range(0, TB, 16)]
        if not head:
            eb = jnp.where(b >= 2, b - 2, NB)
            rowwise = [lambda tk, o=o: epilogue(eb, o, 16, b >= 2, tk) for o in range(0, TB, 16)] + rowwise

        never = zero_s[...]
        st = dict(slot=0, y=None, tok=None, due=[])

        def dense():
            if not mm:
                st["tok"] = None
                return
            f = mm.pop(0)
            st["slot"] += 1
            st["tok"] = None if st["y"] is None else (never, st["y"][0:8])
            if f is None:
                st["y"] = st["y"][st["y"].shape[0] - 8:]
                return
            due = None
            while st["due"] and st["due"][0][0] <= st["slot"]:
                v, store = st["due"].pop(0)[1]
                store()
                due = (never, after(v, due))
            st["y"] = f(due)

        def fill():
            if rowwise:
                st["due"].append((st["slot"] + LAG, rowwise.pop(0)(st["tok"])))

        for c in range(LEAD):
            dense()
            if c % 2 == 1 and not head:
                fill()
        late = []
        sc, linv = {}, {}
        for u in range(len(units) + 1):
            if u < len(units):
                g, a = units[u]
                sc[u] = [qk(b * nq + a, g, j, nprev[a], (u % 2) * 4 + j) for j in range(4)]
                linv[u] = []
            acc = None
            for c in range(6):
                dense()
                if u >= 1:
                    pg, pa = units[u - 1]
                    if c in PV[:nprev[pa] + 1]:
                        acc, v = pv(b * nq + pa, pg, nprev[pa], ((u - 1) % 2) * 4, PV.index(c), acc)
                        if c != PV[2]:
                            st["due"].insert(0, (0, (v, lambda: None)))
                    if c == PV[3]:
                        store = att_out(b * nq + pa, pg, acc, linv.pop(u - 1))
                        if pg == G - 1:
                            late.append(store)
                        else:
                            store()
                for j in range(4):
                    if u < len(units) and c == SM[j]:
                        linv[u].append(softmax(*sc[u][j], (u % 2) * 4 + j, st["tok"]))
                if c in FILL[u % len(FILL)] and (u >= 2 or not head):
                    fill()
        while mm or rowwise:
            dense()
            dense()
            fill()
        for _, (_, store) in st["due"]:
            store()
        for store in late:
            store()

    def tail():
        never = zero_s[...]
        rowwise = [(NB - 2, o) for o in range(0, TB, 16)]
        y, due, n = None, [], 0
        for off in range(0, TB, 64):
            for c0 in range(0, D, 256):
                tok = None if y is None else (never, y[0:8])
                wait = None
                while due and due[0][0] <= n:
                    v, store = due.pop(0)[1]
                    store()
                    wait = (never, after(v, wait))
                y = wo_mm(NB - 1, off, 64, c0, 256, wait)
                for _ in range(2):
                    if rowwise:
                        due.append((n + 3, epilogue(*rowwise.pop(0), 16, None, tok)))
                n += 1
            rowwise += [(NB - 1, off + o) for o in range(0, 64, 16)]
        due += [(0, epilogue(*r, 16)) for r in rowwise]
        for _, (_, store) in due:
            store()

    def routed_token():
        best, bidx = best_s[...], bidx_s[...]
        top = jnp.max(best, axis=0, keepdims=True)
        idx = jnp.min(jnp.where(best == top, bidx, S - 1))
        grp = pl.multiple_of((idx >> 4) << 4, 16)
        x1 = x1_s[pl.ds(grp, 16), :].astype(F32)
        xn = _layernorm(x1).astype(BF16)
        nf = F // 128 // 2

        def half(i, y):
            def cols(w_s):
                return _bf(jnp.concatenate([w_s.bitcast(I32)[i * nf + c] for c in range(nf)], axis=1))

            hid = []
            for c in range(0, nf * 128, 256):
                gate = _rb(jnp.dot(xn, cols(wg_s)[:, c:c + 256], preferred_element_type=F32))
                up = _rb(jnp.dot(xn, cols(wu_s)[:, c:c + 256], preferred_element_type=F32))
                hid.append((_rb(gate * jax.nn.sigmoid(gate)) * up).astype(BF16))
            for c, h in enumerate(hid):
                r = pl.ds(pl.multiple_of(i * (nf * 64) + c * 128, 8), 128)
                wd = jnp.concatenate([wd_s.bitcast(I32)[n, r, :] for n in range(G)], axis=1)
                y = y + jnp.dot(h, _bf(wd), preferred_element_type=F32)
            return y

        y = _rb(lax.fori_loop(0, 2, half, jnp.zeros((16, D), F32)))
        y = _rb(y * _rb(jax.nn.sigmoid(top[:, 0:1])))
        xn = xn.astype(F32)
        sel = lax.broadcasted_iota(I32, (16, D), 0) == (idx & 15)
        x2 = (x1 + jnp.where(sel, _rb(xn + y), xn)).astype(BF16)
        return grp, x2

    zero_s[...] = jnp.zeros((8, 128), I32)
    x1_s[rows(NB), :] = jnp.zeros((TB, D), BF16)
    for c in range(TB // 64):
        arrive(x_cp[c // 2])
        ln_in(0, 64 * c, 64)[1]()
    transpose_wv(0)
    body(0, True, cold=True)
    arrive(queue[-1])

    def layer(li, carry):
        best_s[...] = jnp.full((8, 128), -jnp.inf, F32)
        bidx_s[...] = jnp.zeros((8, 128), I32)

        def step(b, c):
            body(b, False)

            @pl.when(jnp.logical_and(li == 0, b == 1))
            def _():
                x_cp[4].start()

            @pl.when(jnp.logical_and(li == 0, b == 2))
            def _():
                x_cp[4].wait()
                for cp in ffn_cp:
                    cp.start()

            @pl.when(jnp.logical_and(li == 1, b >= 2))
            def _():
                out_cp(b - 2).start()
            return c

        lax.fori_loop(1, NB, step, 0)
        tail()

        @pl.when(li == 0)
        def _():
            for cp in ffn_cp:
                cp.wait()

        @pl.when(li == 1)
        def _():
            out_cp(NB - 2).start()
            out_cp(NB - 1).start()

        grp, x2 = routed_token()

        @pl.when(li == 0)
        def _():
            x_s[pl.ds(grp, 16), :] = x2
            xn = _layernorm(x2.astype(F32)).astype(BF16)
            for g in range(G):
                xn_s[g][pl.ds(grp, 16), :] = xn[:, g * 128:(g + 1) * 128]
            body(0, True)

        @pl.when(li == 1)
        def _():
            for blk in range(NB):
                out_cp(blk).wait()
            x_s[pl.ds(grp, 16), :] = x2
            cp = pltpu.make_async_copy(x_s.at[pl.ds(grp, 16)], out_hbm.at[pl.ds(grp, 16)], sem_o.at[0])
            cp.start()
            cp.wait()

        return carry

    lax.fori_loop(0, 2, layer, 0)


@jax.jit
def pallas_interleave_layers__sliding_block__moe_arch_mod__prompt_kernel(
    A_x: jax.Array,
    A_wqkv: jax.Array,
    A_wo: jax.Array,
    B_x: jax.Array,
    B_w_r: jax.Array,
    B_w_gate: jax.Array,
    B_w_up: jax.Array,
    B_w_down: jax.Array,
):
    del B_x
    hbm = pl.BlockSpec(memory_space=pl.ANY)
    out = pl.pallas_call(
        _kernel,
        out_shape=jax.ShapeDtypeStruct((S, D), BF16),
        in_specs=[hbm, hbm, hbm, pl.BlockSpec(memory_space=pltpu.VMEM), hbm, hbm, hbm],
        out_specs=hbm,
        scratch_shapes=[
            pltpu.VMEM((S + TB, D), BF16),
            pltpu.VMEM((S + TB, D), BF16),
            [pltpu.VMEM((S, 128), BF16)] * G,
            [pltpu.VMEM((S, 128), BF16)] * G,
            [pltpu.VMEM((S, 128), BF16)] * G,
            [pltpu.VMEM((S, 128), BF16)] * G,
            [pltpu.VMEM((S // 2, 128), I32)] * G,
            [pltpu.VMEM((256, 128), BF16)] * 8,
            [pltpu.VMEM((256, 128), BF16)] * 8,
            [pltpu.VMEM((D, 128), BF16)] * (3 * G),
            [pltpu.VMEM((D, 128), BF16)] * G,
            [pltpu.VMEM((D, 128), BF16)] * G,
            pltpu.VMEM((F // 128, D, 128), BF16),
            pltpu.VMEM((F // 128, D, 128), BF16),
            pltpu.VMEM((G, F, 128), BF16),
            pltpu.VMEM((8, 128), F32),
            pltpu.VMEM((8, 128), I32),
            pltpu.VMEM((8, 128), I32),
            pltpu.SemaphoreType.DMA((5,)),
            pltpu.SemaphoreType.DMA((4 * G,)),
            pltpu.SemaphoreType.DMA((1,)),
            pltpu.SemaphoreType.DMA((1,)),
        ],
        compiler_params=pltpu.CompilerParams(vmem_limit_bytes=100 * 1024 * 1024),
    )(A_x.reshape(S, D), A_wqkv, A_wo, B_w_r, B_w_gate, B_w_up, B_w_down)
    return out.reshape(1, S, D)
```

```python
import jax
import jax.numpy as jnp
from jax import lax
import jax.experimental.pallas as pl
import jax.experimental.pallas.tpu as pltpu

F32 = jnp.float32
BF16 = jnp.bfloat16
I32 = jnp.int32

S, D, F = 2048, 1024, 3584
TB = 256
NB = S // TB
MC = 128
LEAD = 14
SM = (0, 2, 4, 5)
PV = (2, 3, 4, 5)
FILL = ((1, 5), (1,))
LAG = 5
TLAG = 5
DLAG = 2
AHEAD = (5, 12)
WAITS = (0, 1, 2, 4, 6, 8)
G = D // 128
SCALE = 0.1767578125
LOG2E = 1.4426950408889634
EPS = 1.0013580322265625e-05
NT = (((1,), (1,)), ((), ()))


def _rb(x):
    return x.astype(BF16).astype(F32)


def _ld(ref, lead, start, size):
    return ref[lead].bitcast(I32)[pl.ds(start // 2, size // 2), :]


def _bf(words):
    return pltpu.bitcast(words, BF16)


def _seg(rows):
    return lax.broadcasted_iota(I32, (rows, 128), 1) >> 5


def _layernorm(x):
    m = jnp.sum(x, axis=-1, keepdims=True) * (1.0 / D)
    c = x - m
    v = jnp.sum(c * c, axis=-1, keepdims=True) * (1.0 / D)
    den = _rb(jnp.sqrt(_rb(_rb(v) + EPS)))
    return _rb(x - _rb(m)) * (1.0 / den)


def _butterfly(tiles, starts):
    def comb(a, sa, b, sb, bit, want):
        ea, eb = sa + a.shape[0], sb + b.shape[0]
        cuts = sorted({sa, ea, sb, eb})
        parts = []
        for lo, hi in zip(cuts[:-1], cuts[1:]):
            take_a = ((_seg(hi - lo) >> bit) & 1) == want
            xa = a[lo - sa:hi - sa] if sa <= lo and hi <= ea else 0
            xb = b[lo - sb:hi - sb] if sb <= lo and hi <= eb else 0
            parts.append(jnp.where(take_a, xa, xb))
        return (jnp.concatenate(parts, axis=0) if len(parts) > 1 else parts[0]), cuts[0]

    st = {}
    for j1 in range(2):
        for h0 in range(2):
            st[j1, h0] = comb(tiles[2 * j1], starts[2 * j1], tiles[2 * j1 + 1], starts[2 * j1 + 1], 0, h0)
    return [comb(*st[0, h & 1], *st[1, h & 1], 1, h >> 1)[0] for h in range(4)]


def _kernel(x_hbm, wqkv_hbm, wo_hbm, wr_ref, wg_hbm, wu_hbm, wd_hbm, out_hbm,
            x_s, x1_s, xn_s, q_s, k_s, vt_s, o_s, s_s, p_s, wqkv_s, wvt_s, wo_s, wg_s, wu_s, wd_s,
            best_s, bidx_s, zero_s, col_s, sem_x, sem_w, sem_f, sem_o):

    def rows(blk, off=0, size=TB):
        return pl.ds(pl.multiple_of(blk * TB + off, 16), size)

    x_cp = [pltpu.make_async_copy(x_hbm.at[pl.ds(lo, n)], x_s.at[pl.ds(lo, n)], sem_x.at[i])
            for i, (lo, n) in enumerate(((0, 128), (128, TB - 128), (TB, TB), (2 * TB, 2 * TB), (4 * TB, S - 4 * TB)))]
    w_cp = [pltpu.make_async_copy(wqkv_hbm.at[:, pl.ds(c * 128, 128)], wqkv_s[c], sem_w.at[c])
            for c in range(3 * G)]
    wo_cp = [pltpu.make_async_copy(wo_hbm.at[:, pl.ds(c * 128, 128)], wo_s[c], sem_w.at[3 * G + c])
             for c in range(G)]
    ffn_cp = [pltpu.make_async_copy(src.at[:, pl.ds(c * 128, 128)], dst.at[c], sem_f.at[0])
              for src, dst in ((wg_hbm, wg_s), (wu_hbm, wu_s), (wd_hbm, wd_s)) for c in range(dst.shape[0])]

    def out_cp(blk):
        return pltpu.make_async_copy(x_s.at[rows(blk)], out_hbm.at[rows(blk)], sem_o.at[0])

    queue = [x_cp[0], w_cp[2 * G], x_cp[1]]
    for g in range(G):
        queue += [w_cp[G + g], w_cp[g]] + w_cp[2 * G + g + 1:2 * G + g + 2] + ([x_cp[2]] if g == 1 else [])
    queue += wo_cp + [x_cp[3]]
    flight = dict(started=0, waited=0)

    def launch():
        ahead = min(AHEAD[0] + flight["waited"], AHEAD[1])
        while flight["started"] < min(flight["waited"] + ahead, len(queue)):
            queue[flight["started"]].start()
            flight["started"] += 1

    def arrive(cp):
        n = next(i for i, c in enumerate(queue) if c is cp) + 1
        while flight["waited"] < n:
            queue[flight["waited"]].wait()
            flight["waited"] += 1
            launch()

    def transpose_wv(g):
        for c in range(G):
            wvt_s[c][pl.ds(g * 128, 128), :] = wqkv_s[2 * G + g][pl.ds(c * 128, 128), :].T

    r32 = lax.broadcasted_iota(I32, (32, 128), 0)
    first = r32 > (lax.broadcasted_iota(I32, (32, 128), 1) & 31)
    r16 = lax.broadcasted_iota(I32, (16, 128), 0)
    t16 = lax.broadcasted_iota(I32, (16, 128), 1) & 31
    first_w = jnp.where(2 * r16 > t16, 0xFFFF, 0) | jnp.where(2 * r16 + 1 > t16, -65536, 0)

    def after(x, tok):
        if tok is None:
            return x
        never, val = tok
        reps = (x.shape[0] // 8, x.shape[1] // 128)
        val = lax.bitcast_convert_type(val, x.dtype)
        return jnp.where(jnp.tile(never, reps) < 0, jnp.tile(val, reps), x)

    def words_after(w, tok):
        if tok is None:
            return w
        return jnp.concatenate([after(w[0:8], tok), w[8:]], axis=0)

    def ln_in(blk, off, size, tok=None):
        xf = _layernorm(after(x_s[rows(blk, off, size), :].astype(F32), tok))
        xn = xf.astype(BF16)

        def store():
            for g in range(G):
                xn_s[g][rows(blk, off, size), :] = xn[:, g * 128:(g + 1) * 128]

        return xf[size - 8:, D - 128:], store

    def xn_rows(blk, off, size, tok=None):
        return _bf(join([_ld(xn_s, t, blk * TB + off, size) for t in range(G)], tok))

    def join(slabs, tok):
        return jnp.concatenate([words_after(w, tok if t < 1 else None) for t, w in enumerate(slabs)], axis=1)

    def proj_qk(blk, g, which, off, size, tok):
        w = _bf(_ld(wqkv_s, which * G + g, 0, D))
        y = jnp.dot(xn_rows(blk, off, size, tok), w, preferred_element_type=F32)
        (q_s, k_s)[which][g][rows(blk, off, size), :] = y.astype(BF16)
        return y

    def proj_v(blk, g, t, tok):
        wvt = _bf(join([_ld(wvt_s, c, g * 128, 128) for c in range(G)], tok))
        vt = lax.dot_general(wvt, xn_rows(blk, 128 * t, 128), NT, preferred_element_type=F32)
        vt_s[g][rows(blk, 128 * t, 128), :] = vt.astype(BF16)
        return vt

    def qk(i, g, j, nprev, slot):
        q = _ld(q_s, g, i * 128 + 32 * j, 32)
        w = jnp.concatenate([jnp.where(_seg(16) == (s ^ j), q, 0) for s in range(4)], axis=0)
        if nprev == 2:
            k = _ld(k_s, g, i * 128 + 32 * j - 256, 288)
        else:
            k = _ld(k_s, g, 0, nprev * 128 + 32 * j + 32)
        s = lax.dot_general(_bf(k), _bf(w), NT, preferred_element_type=F32)
        n = s.shape[0]
        if nprev == 2:
            sm = jnp.concatenate([jnp.where(first, s[0:32], s[256:288]), s[32:256]], axis=0)
        else:
            sm = jnp.where(first, -jnp.inf, s[n - 32:n])
            if n > 32:
                sm = jnp.concatenate([sm, s[0:n - 32]], axis=0)
        mx = jnp.broadcast_to(jnp.max(sm, axis=0, keepdims=True), (8, 128))
        s_s[slot][pl.ds(0, sm.shape[0]), :] = sm.astype(BF16)
        return sm.shape[0], _rb(mx)

    def softmax(m, mx, slot, tok):
        sm = _bf(_ld(s_s, slot, 0, m)).astype(F32)
        p = jnp.exp2((sm - jnp.tile(after(mx, tok), (m // 8, 1))) * (SCALE * LOG2E))
        l = jnp.sum(p, axis=0, keepdims=True)
        p_s[slot][pl.ds(0, m), :] = p.astype(BF16)
        return jnp.broadcast_to(1.0 / _rb(l), (8, 128))

    def p_words(slot, j, nprev, lo, hi):
        n = 144 if nprev == 2 else nprev * 64 + 16 * j + 16
        parts = []
        for r in range(lo, hi, 16):
            if r == n - 16:
                w = _ld(p_s, slot, 0, 32)
                parts.append(w & ~first_w if nprev == 2 else w)
            elif nprev == 2:
                w = _ld(p_s, slot, 2 * r, 32)
                parts.append(w & first_w if r == 0 else w)
            else:
                parts.append(_ld(p_s, slot, 2 * r + 32, 32))
        return jnp.concatenate(parts, axis=0) if len(parts) > 1 else parts[0]

    def pv(i, g, nprev, slot, t, acc):
        tiles, starts = [], []
        for j in range(4):
            st = 16 * j if nprev == 2 else 0
            n = 144 if nprev == 2 else nprev * 64 + 16 * j + 16
            lo, hi = max(64 * t, st), min(64 * t + 64, st + n)
            tiles.append(p_words(slot + j, j, nprev, lo - st, hi - st))
            starts.append(lo)
        p = _butterfly(tiles, starts)
        out = []
        for h in range(4):
            v = _ld(vt_s, g, (i - nprev + t) * 128 + 32 * h, 32)
            r = jnp.dot(_bf(v), _bf(p[h]), preferred_element_type=F32)
            out.append(r if acc is None else acc[h] + r)
        return out, p[3][0:8]

    def att_out(i, g, acc, linv):
        linv = _butterfly(linv, [0] * 4)
        o = jnp.concatenate([acc[h] * jnp.concatenate([linv[h]] * 4, axis=0) for h in range(4)], axis=0)
        o = pltpu.bitcast(o.astype(BF16).T, I32)
        b = [o[16 * s:16 * s + 16] for s in range(4)]
        b = [jnp.where((_seg(16) & 1) == 0, b[s], b[s ^ 1]) for s in range(4)]
        b = [jnp.where((_seg(16) & 2) == 0, b[s], b[s ^ 2]) for s in range(4)]

        def store():
            o_s[g][pl.ds(pl.multiple_of(i * 64, 8), 64), :] = jnp.concatenate(b, axis=0)

        return store

    def wo_mm(blk, off, size, c0=0, cn=D, tok=None):
        o = _bf(join(
            [o_s[t][pl.ds(pl.multiple_of((blk * TB + off) // 2, 8), size // 2), :] for t in range(G)], tok))
        a = jnp.dot(o, _bf(jnp.concatenate([_ld(wo_s, c, 0, D) for c in range(c0 // 128, (c0 + cn) // 128)], axis=1)), preferred_element_type=F32)
        x = x_s[rows(blk, off, size), c0:c0 + cn].astype(F32)
        x1_s[rows(blk, off, size), c0:c0 + cn] = (x + _rb(a)).astype(BF16)
        return a[:, 0:128]

    def epilogue(blk, off, size, valid=None, tok=None):
        x1 = after(x1_s[rows(blk, off, size), :].astype(F32), tok)
        xn = _rb(_layernorm(x1))
        x2 = (x1 + (xn + xn * 0.0)).astype(BF16)
        r = _rb(jnp.sum(xn * wr_ref[...].astype(F32).reshape(1, D), axis=-1, keepdims=True))
        if valid is not None:
            r = jnp.where(valid, r, -jnp.inf)
        best, bidx = best_s[...], bidx_s[...]
        pos = lax.broadcasted_iota(I32, (8, 128), 0) + (blk * TB + off)
        for t in range(size // 8):
            rt = jnp.broadcast_to(r[8 * t:8 * t + 8], (8, 128))
            up = rt > best
            best = jnp.where(up, rt, best)
            bidx = jnp.where(up, pos + 8 * t, bidx)
        best_s[...] = best
        bidx_s[...] = bidx

        def store():
            x_s[rows(blk, off, size), :] = x2

        return best, store

    def body(b, head, cold=False):
        nq = TB // 128
        units = [(g, a) for g in range(G) for a in range(nq)]
        nprev = [min(a, 2) if head else 2 for a in range(nq)]
        nxt = 1 if head else lax.rem(b + 1, NB)

        def qk_task(tk, g, w, o):
            if cold and o == 0 and w == 1 and g in WAITS:
                upto = WAITS[WAITS.index(g) + 1]
                arrive(w_cp[2 * G + upto] if upto < G else w_cp[G - 1])
            return proj_qk(b, g, w, o, MC, tk)

        def v_task(tk, g, t):
            y = proj_v(b, g, t, tk)
            if cold and t == 0 and g + 1 < G:
                transpose_wv(g + 1)
            return y

        def ln_task(tk, o):
            if cold and o == 0:
                arrive(x_cp[2])
            return ln_in(nxt, o, 16, tk)

        mm = []
        for g in range(G):
            for t in range(nq):
                for which in (1, 0):
                    for off in range(0, 128, MC):
                        mm.append(lambda tk, g=g, w=which, o=128 * t + off: qk_task(tk, g, w, o))
                        mm.extend([None] * (MC // 64 - 1))
                mm.extend([lambda tk, g=g, t=t: v_task(tk, g, t), None])
        if not head:
            for off in range(0, TB, MC):
                for c in range(G):
                    mm.append(lambda tk, o=off, c=c: wo_mm(b - 1, o, MC, 128 * c, 128, tk))
                    mm.extend([None] * (MC // 64 - 1))
        rowwise = [lambda tk, o=o: ln_task(tk, o) for o in range(0, TB, 16)]
        if not head:
            eb = jnp.where(b >= 2, b - 2, NB)
            rowwise = [lambda tk, o=o: epilogue(eb, o, 16, b >= 2, tk) for o in range(0, TB, 16)] + rowwise

        never = zero_s[...]
        st = dict(slot=0, y=None, tok=None, due=[])

        def dense():
            if not mm:
                st["tok"] = None
                return
            f = mm.pop(0)
            st["slot"] += 1
            st["tok"] = None if st["y"] is None else (never, st["y"][0:8])
            if f is None:
                st["y"] = st["y"][st["y"].shape[0] - 8:]
                return
            due = None
            while st["due"] and st["due"][0][0] <= st["slot"]:
                v, store = st["due"].pop(0)[1]
                store()
                due = (never, after(v, due))
            st["y"] = f(due)

        def fill(extra=0):
            if rowwise:
                st["due"].append((st["slot"] + LAG + extra, rowwise.pop(0)(st["tok"])))

        for c in range(LEAD):
            dense()
            if c % 2 == 1 and not head:
                fill()
        late = []
        sc, linv = {}, {}
        for u in range(len(units) + 1):
            if u < len(units):
                g, a = units[u]
                sc[u] = [qk(b * nq + a, g, j, nprev[a], (u % 2) * 4 + j) for j in range(4)]
                linv[u] = []
            acc = None
            for c in range(6):
                dense()
                if u >= 1:
                    pg, pa = units[u - 1]
                    if c in PV[:nprev[pa] + 1]:
                        acc, v = pv(b * nq + pa, pg, nprev[pa], ((u - 1) % 2) * 4, PV.index(c), acc)
                        if c != PV[2]:
                            st["due"].insert(0, (0, (v, lambda: None)))
                    if c == PV[3]:
                        store = att_out(b * nq + pa, pg, acc, linv.pop(u - 1))
                        if pg == G - 1:
                            late.append(store)
                        else:
                            store()
                for j in range(4):
                    if u < len(units) and c == SM[j]:
                        linv[u].append(softmax(*sc[u][j], (u % 2) * 4 + j, st["tok"]))
                if c in FILL[u % len(FILL)] and (u >= 2 or not head):
                    fill()
        while mm or rowwise:
            dense()
            fill(2)
            dense()
        for _, (_, store) in st["due"]:
            store()
        for store in late:
            store()

    def tail():
        never = zero_s[...]
        rowwise = [(NB - 2, o) for o in range(0, TB, 16)]
        y, due, n = None, [], 0
        for off in range(0, TB, 64):
            for c0 in range(0, D, 256):
                tok = None if y is None else (never, y[0:8])
                wait = None
                while due and due[0][0] <= n:
                    v, store = due.pop(0)[1]
                    store()
                    wait = (never, after(v, wait))
                y = wo_mm(NB - 1, off, 64, c0, 256, wait)
                for _ in range(2):
                    if rowwise:
                        due.append((n + TLAG, epilogue(*rowwise.pop(0), 16, None, tok)))
                n += 1
            rowwise += [(NB - 1, off + o) for o in range(0, 64, 16)]
        due += [(0, epilogue(*r, 16)) for r in rowwise]
        for _, (_, store) in due:
            store()

    def routed_token():
        best, bidx = best_s[...], bidx_s[...]
        top = jnp.max(best, axis=0, keepdims=True)
        idx = jnp.min(jnp.where(best == top, bidx, S - 1))
        grp = pl.multiple_of((idx >> 4) << 4, 16)
        x1 = x1_s[pl.ds(grp, 16), :].astype(F32)
        xn = _layernorm(x1).astype(BF16)
        sel = lax.broadcasted_iota(I32, (16, D), 0) == (idx & 15)
        row = jnp.sum(jnp.where(sel, xn.astype(F32), 0.0), axis=0, keepdims=True)
        for c in range(G):
            col_s[pl.ds(c * 128, 128), :] = jnp.broadcast_to(row[:, c * 128:(c + 1) * 128], (128, 128)).T

        y, hid = None, []
        for c in range(F // 256 + DLAG):
            if c < F // 256:
                wg = jnp.concatenate([wg_s.bitcast(I32)[2 * c + n] for n in range(2)], axis=1)
                gate = _rb(jnp.dot(xn, _bf(wg), preferred_element_type=F32))
                up = [0.0, 0.0]
                for r in range(0, D, 16):
                    col = col_s[pl.ds(r, 16), :]
                    for n in range(2):
                        w = _bf(wu_s.bitcast(I32)[2 * c + n, pl.ds(r // 2, 8), :]).astype(F32)
                        up[n] = up[n] + w * col
                up = _rb(jnp.sum(jnp.concatenate(up, axis=1), axis=0, keepdims=True))
                hid.append((_rb(gate * jax.nn.sigmoid(gate)) * up).astype(BF16))
            if c >= DLAG:
                r = pl.ds((c - DLAG) * 128, 128)
                wd = jnp.concatenate([wd_s.bitcast(I32)[n, r, :] for n in range(G)], axis=1)
                part = jnp.dot(hid[c - DLAG], _bf(wd), preferred_element_type=F32)
                y = part if y is None else y + part
        y = _rb(y)
        y = _rb(y * _rb(jax.nn.sigmoid(top[:, 0:1])))
        xn = xn.astype(F32)
        zero = xn * 0.0
        x2 = (x1 + _rb(xn + jnp.where(sel, zero + y, zero))).astype(BF16)
        return grp, x2

    launch()
    zero_s[...] = jnp.zeros((8, 128), I32)
    x1_s[rows(NB), :] = jnp.zeros((TB, D), BF16)
    for c in range(TB // 64):
        arrive(x_cp[c // 2])
        ln_in(0, 64 * c, 64)[1]()
    transpose_wv(0)
    body(0, True, cold=True)
    arrive(queue[-1])

    def layer(li, carry):
        best_s[...] = jnp.full((8, 128), -jnp.inf, F32)
        bidx_s[...] = jnp.zeros((8, 128), I32)

        def step(b, c):
            body(b, False)

            @pl.when(jnp.logical_and(li == 0, b == 1))
            def _():
                x_cp[4].start()

            @pl.when(jnp.logical_and(li == 0, b == 2))
            def _():
                x_cp[4].wait()
                for cp in ffn_cp:
                    cp.start()

            @pl.when(jnp.logical_and(li == 1, b >= 2))
            def _():
                out_cp(b - 2).start()
            return c

        lax.fori_loop(1, NB, step, 0)
        tail()

        @pl.when(li == 0)
        def _():
            for cp in ffn_cp:
                cp.wait()

        @pl.when(li == 1)
        def _():
            out_cp(NB - 2).start()
            out_cp(NB - 1).start()

        grp, x2 = routed_token()

        @pl.when(li == 0)
        def _():
            x_s[pl.ds(grp, 16), :] = x2
            xn = _layernorm(x2.astype(F32)).astype(BF16)
            for g in range(G):
                xn_s[g][pl.ds(grp, 16), :] = xn[:, g * 128:(g + 1) * 128]
            body(0, True)

        @pl.when(li == 1)
        def _():
            for blk in range(NB):
                out_cp(blk).wait()
            x_s[pl.ds(grp, 16), :] = x2
            cp = pltpu.make_async_copy(x_s.at[pl.ds(grp, 16)], out_hbm.at[pl.ds(grp, 16)], sem_o.at[0])
            cp.start()
            cp.wait()

        return carry

    lax.fori_loop(0, 2, layer, 0)


@jax.jit
def pallas_interleave_layers__sliding_block__moe_arch_mod__prompt_kernel(
    A_x: jax.Array,
    A_wqkv: jax.Array,
    A_wo: jax.Array,
    B_x: jax.Array,
    B_w_r: jax.Array,
    B_w_gate: jax.Array,
    B_w_up: jax.Array,
    B_w_down: jax.Array,
):
    del B_x
    hbm = pl.BlockSpec(memory_space=pl.ANY)
    out = pl.pallas_call(
        _kernel,
        out_shape=jax.ShapeDtypeStruct((S, D), BF16),
        in_specs=[hbm, hbm, hbm, pl.BlockSpec(memory_space=pltpu.VMEM), hbm, hbm, hbm],
        out_specs=hbm,
        scratch_shapes=[
            pltpu.VMEM((S + TB, D), BF16),
            pltpu.VMEM((S + TB, D), BF16),
            [pltpu.VMEM((S, 128), BF16)] * G,
            [pltpu.VMEM((S, 128), BF16)] * G,
            [pltpu.VMEM((S, 128), BF16)] * G,
            [pltpu.VMEM((S, 128), BF16)] * G,
            [pltpu.VMEM((S // 2, 128), I32)] * G,
            [pltpu.VMEM((256, 128), BF16)] * 8,
            [pltpu.VMEM((256, 128), BF16)] * 8,
            [pltpu.VMEM((D, 128), BF16)] * (3 * G),
            [pltpu.VMEM((D, 128), BF16)] * G,
            [pltpu.VMEM((D, 128), BF16)] * G,
            pltpu.VMEM((F // 128, D, 128), BF16),
            pltpu.VMEM((F // 128, D, 128), BF16),
            pltpu.VMEM((G, F, 128), BF16),
            pltpu.VMEM((8, 128), F32),
            pltpu.VMEM((8, 128), I32),
            pltpu.VMEM((8, 128), I32),
            pltpu.VMEM((D, 128), F32),
            pltpu.SemaphoreType.DMA((5,)),
            pltpu.SemaphoreType.DMA((4 * G,)),
            pltpu.SemaphoreType.DMA((1,)),
            pltpu.SemaphoreType.DMA((1,)),
        ],
        compiler_params=pltpu.CompilerParams(vmem_limit_bytes=100 * 1024 * 1024),
    )(A_x.reshape(S, D), A_wqkv, A_wo, B_w_r, B_w_gate, B_w_up, B_w_down)
    return out.reshape(1, S, D)
```

```python
import jax
import jax.numpy as jnp
from jax import lax
import jax.experimental.pallas as pl
import jax.experimental.pallas.tpu as pltpu

F32 = jnp.float32
BF16 = jnp.bfloat16
I32 = jnp.int32

S, D, F = 2048, 1024, 3584
TB = 256
NB = S // TB
MC = 128
LEAD = 14
SM = (0, 2, 4, 5)
PV = (2, 3, 4, 5)
FILL = ((1, 5), (1,))
LAG = 5
TLAG = 5
DLAG = 2
AHEAD = 4
WAITS = (0, 1, 2, 3, 4, 6, 8)
G = D // 128
SCALE = 0.1767578125
LOG2E = 1.4426950408889634
EPS = 1.0013580322265625e-05
NT = (((1,), (1,)), ((), ()))


def _rb(x):
    return x.astype(BF16).astype(F32)


def _ld(ref, lead, start, size):
    return ref[lead].bitcast(I32)[pl.ds(start // 2, size // 2), :]


def _bf(words):
    return pltpu.bitcast(words, BF16)


def _seg(rows):
    return lax.broadcasted_iota(I32, (rows, 128), 1) >> 5


def _layernorm(x):
    m = jnp.sum(x, axis=-1, keepdims=True) * (1.0 / D)
    c = x - m
    v = jnp.sum(c * c, axis=-1, keepdims=True) * (1.0 / D)
    den = _rb(jnp.sqrt(_rb(_rb(v) + EPS)))
    return _rb(x - _rb(m)) * (1.0 / den)


def _butterfly(tiles, starts):
    def comb(a, sa, b, sb, bit, want):
        ea, eb = sa + a.shape[0], sb + b.shape[0]
        cuts = sorted({sa, ea, sb, eb})
        parts = []
        for lo, hi in zip(cuts[:-1], cuts[1:]):
            take_a = ((_seg(hi - lo) >> bit) & 1) == want
            xa = a[lo - sa:hi - sa] if sa <= lo and hi <= ea else 0
            xb = b[lo - sb:hi - sb] if sb <= lo and hi <= eb else 0
            parts.append(jnp.where(take_a, xa, xb))
        return (jnp.concatenate(parts, axis=0) if len(parts) > 1 else parts[0]), cuts[0]

    st = {}
    for j1 in range(2):
        for h0 in range(2):
            st[j1, h0] = comb(tiles[2 * j1], starts[2 * j1], tiles[2 * j1 + 1], starts[2 * j1 + 1], 0, h0)
    return [comb(*st[0, h & 1], *st[1, h & 1], 1, h >> 1)[0] for h in range(4)]


def _kernel(x_hbm, wqkv_hbm, wo_hbm, wr_ref, wg_hbm, wu_hbm, wd_hbm, out_hbm,
            x_s, x1_s, xn_s, q_s, k_s, vt_s, o_s, s_s, p_s, wqkv_s, wvt_s, wo_s, wg_s, wu_s, wd_s,
            best_s, bidx_s, zero_s, col_s, sem_x, sem_w, sem_f, sem_o):

    def rows(blk, off=0, size=TB):
        return pl.ds(pl.multiple_of(blk * TB + off, 16), size)

    x_cp = [pltpu.make_async_copy(x_hbm.at[pl.ds(lo, n)], x_s.at[pl.ds(lo, n)], sem_x.at[i])
            for i, (lo, n) in enumerate(((0, 128), (128, TB - 128), (TB, TB), (2 * TB, TB), (3 * TB, S - 3 * TB)))]
    w_cp = [pltpu.make_async_copy(wqkv_hbm.at[:, pl.ds(c * 128, 128)], wqkv_s[c], sem_w.at[c])
            for c in range(3 * G)]
    wo_cp = [pltpu.make_async_copy(wo_hbm.at[:, pl.ds(c * 128, 128)], wo_s[c], sem_w.at[3 * G + c])
             for c in range(G)]
    ffn_cp = [pltpu.make_async_copy(src.at[:, pl.ds(c * 128, 128)], dst.at[c], sem_f.at[0])
              for src, dst in ((wg_hbm, wg_s), (wu_hbm, wu_s), (wd_hbm, wd_s)) for c in range(dst.shape[0])]

    def out_cp(blk):
        return pltpu.make_async_copy(x_s.at[rows(blk)], out_hbm.at[rows(blk)], sem_o.at[0])

    queue = [x_cp[0], w_cp[2 * G], x_cp[1]]
    for g in range(G):
        queue += [w_cp[G + g], w_cp[g]] + w_cp[2 * G + g + 1:2 * G + g + 2] + ([x_cp[2]] if g == 1 else [])
    queue += wo_cp + [x_cp[3]]
    flight = dict(started=0, waited=0)

    def launch(more=0):
        upto = max(flight["waited"] + AHEAD, flight["started"] + more)
        while flight["started"] < min(upto, len(queue)):
            queue[flight["started"]].start()
            flight["started"] += 1

    def arrive(cp):
        n = next(i for i, c in enumerate(queue) if c is cp) + 1
        while flight["waited"] < n:
            queue[flight["waited"]].wait()
            flight["waited"] += 1
            launch()

    def transpose_wv(g):
        for c in range(G):
            wvt_s[c][pl.ds(g * 128, 128), :] = wqkv_s[2 * G + g][pl.ds(c * 128, 128), :].T

    r32 = lax.broadcasted_iota(I32, (32, 128), 0)
    first = r32 > (lax.broadcasted_iota(I32, (32, 128), 1) & 31)
    r16 = lax.broadcasted_iota(I32, (16, 128), 0)
    t16 = lax.broadcasted_iota(I32, (16, 128), 1) & 31
    first_w = jnp.where(2 * r16 > t16, 0xFFFF, 0) | jnp.where(2 * r16 + 1 > t16, -65536, 0)

    def after(x, tok):
        if tok is None:
            return x
        never, val = tok
        reps = (x.shape[0] // 8, x.shape[1] // 128)
        val = lax.bitcast_convert_type(val, x.dtype)
        return jnp.where(jnp.tile(never, reps) < 0, jnp.tile(val, reps), x)

    def words_after(w, tok):
        if tok is None:
            return w
        return jnp.concatenate([after(w[0:8], tok), w[8:]], axis=0)

    def ln_in(blk, off, size, tok=None):
        xf = _layernorm(after(x_s[rows(blk, off, size), :].astype(F32), tok))
        xn = xf.astype(BF16)

        def store():
            for g in range(G):
                xn_s[g][rows(blk, off, size), :] = xn[:, g * 128:(g + 1) * 128]

        return xf[size - 8:, D - 128:], store

    def xn_rows(blk, off, size, tok=None):
        return _bf(join([_ld(xn_s, t, blk * TB + off, size) for t in range(G)], tok))

    def join(slabs, tok):
        return jnp.concatenate([words_after(w, tok if t < 1 else None) for t, w in enumerate(slabs)], axis=1)

    def proj_qk(blk, g, which, off, size, tok):
        w = _bf(_ld(wqkv_s, which * G + g, 0, D))
        y = jnp.dot(xn_rows(blk, off, size, tok), w, preferred_element_type=F32)
        (q_s, k_s)[which][g][rows(blk, off, size), :] = y.astype(BF16)
        return y

    def proj_v(blk, g, t, tok):
        wvt = _bf(join([_ld(wvt_s, c, g * 128, 128) for c in range(G)], tok))
        vt = lax.dot_general(wvt, xn_rows(blk, 128 * t, 128), NT, preferred_element_type=F32)
        vt_s[g][rows(blk, 128 * t, 128), :] = vt.astype(BF16)
        return vt

    def qk(i, g, j, nprev, slot):
        q = _ld(q_s, g, i * 128 + 32 * j, 32)
        w = jnp.concatenate([jnp.where(_seg(16) == (s ^ j), q, 0) for s in range(4)], axis=0)
        if nprev == 2:
            k = _ld(k_s, g, i * 128 + 32 * j - 256, 288)
        else:
            k = _ld(k_s, g, 0, nprev * 128 + 32 * j + 32)
        s = lax.dot_general(_bf(k), _bf(w), NT, preferred_element_type=F32)
        n = s.shape[0]
        if nprev == 2:
            sm = jnp.concatenate([jnp.where(first, s[0:32], s[256:288]), s[32:256]], axis=0)
        else:
            sm = jnp.where(first, -jnp.inf, s[n - 32:n])
            if n > 32:
                sm = jnp.concatenate([sm, s[0:n - 32]], axis=0)
        mx = jnp.broadcast_to(jnp.max(sm, axis=0, keepdims=True), (8, 128))
        s_s[slot][pl.ds(0, sm.shape[0]), :] = sm.astype(BF16)
        return sm.shape[0], _rb(mx)

    def softmax(m, mx, slot, tok):
        sm = _bf(_ld(s_s, slot, 0, m)).astype(F32)
        p = jnp.exp2((sm - jnp.tile(after(mx, tok), (m // 8, 1))) * (SCALE * LOG2E))
        l = jnp.sum(p, axis=0, keepdims=True)
        p_s[slot][pl.ds(0, m), :] = p.astype(BF16)
        return jnp.broadcast_to(1.0 / _rb(l), (8, 128))

    def p_words(slot, j, nprev, lo, hi):
        n = 144 if nprev == 2 else nprev * 64 + 16 * j + 16
        parts = []
        for r in range(lo, hi, 16):
            if r == n - 16:
                w = _ld(p_s, slot, 0, 32)
                parts.append(w & ~first_w if nprev == 2 else w)
            elif nprev == 2:
                w = _ld(p_s, slot, 2 * r, 32)
                parts.append(w & first_w if r == 0 else w)
            else:
                parts.append(_ld(p_s, slot, 2 * r + 32, 32))
        return jnp.concatenate(parts, axis=0) if len(parts) > 1 else parts[0]

    def pv(i, g, nprev, slot, t, acc):
        tiles, starts = [], []
        for j in range(4):
            st = 16 * j if nprev == 2 else 0
            n = 144 if nprev == 2 else nprev * 64 + 16 * j + 16
            lo, hi = max(64 * t, st), min(64 * t + 64, st + n)
            tiles.append(p_words(slot + j, j, nprev, lo - st, hi - st))
            starts.append(lo)
        p = _butterfly(tiles, starts)
        out = []
        for h in range(4):
            v = _ld(vt_s, g, (i - nprev + t) * 128 + 32 * h, 32)
            r = jnp.dot(_bf(v), _bf(p[h]), preferred_element_type=F32)
            out.append(r if acc is None else acc[h] + r)
        return out, p[3][0:8]

    def att_out(i, g, acc, linv):
        linv = _butterfly(linv, [0] * 4)
        o = jnp.concatenate([acc[h] * jnp.concatenate([linv[h]] * 4, axis=0) for h in range(4)], axis=0)
        o = pltpu.bitcast(o.astype(BF16).T, I32)
        b = [o[16 * s:16 * s + 16] for s in range(4)]
        b = [jnp.where((_seg(16) & 1) == 0, b[s], b[s ^ 1]) for s in range(4)]
        b = [jnp.where((_seg(16) & 2) == 0, b[s], b[s ^ 2]) for s in range(4)]

        def store():
            o_s[g][pl.ds(pl.multiple_of(i * 64, 8), 64), :] = jnp.concatenate(b, axis=0)

        return store

    def wo_mm(blk, off, size, c0=0, cn=D, tok=None):
        o = _bf(join(
            [o_s[t][pl.ds(pl.multiple_of((blk * TB + off) // 2, 8), size // 2), :] for t in range(G)], tok))
        a = jnp.dot(o, _bf(jnp.concatenate([_ld(wo_s, c, 0, D) for c in range(c0 // 128, (c0 + cn) // 128)], axis=1)), preferred_element_type=F32)
        x = x_s[rows(blk, off, size), c0:c0 + cn].astype(F32)
        x1_s[rows(blk, off, size), c0:c0 + cn] = (x + _rb(a)).astype(BF16)
        return a[:, 0:128]

    def epilogue(blk, off, size, valid=None, tok=None):
        x1 = after(x1_s[rows(blk, off, size), :].astype(F32), tok)
        xn = _rb(_layernorm(x1))
        x2 = (x1 + (xn + xn * 0.0)).astype(BF16)
        r = _rb(jnp.sum(xn * wr_ref[...].astype(F32).reshape(1, D), axis=-1, keepdims=True))
        if valid is not None:
            r = jnp.where(valid, r, -jnp.inf)
        best, bidx = best_s[...], bidx_s[...]
        pos = lax.broadcasted_iota(I32, (8, 128), 0) + (blk * TB + off)
        for t in range(size // 8):
            rt = jnp.broadcast_to(r[8 * t:8 * t + 8], (8, 128))
            up = rt > best
            best = jnp.where(up, rt, best)
            bidx = jnp.where(up, pos + 8 * t, bidx)
        best_s[...] = best
        bidx_s[...] = bidx

        def store():
            x_s[rows(blk, off, size), :] = x2

        return best, store

    def body(b, head, cold=False):
        nq = TB // 128
        units = [(g, a) for g in range(G) for a in range(nq)]
        nprev = [min(a, 2) if head else 2 for a in range(nq)]
        nxt = 1 if head else lax.rem(b + 1, NB)

        def qk_task(tk, g, w, o):
            if cold and o == 0 and w == 1 and g in WAITS:
                upto = WAITS[WAITS.index(g) + 1]
                arrive(w_cp[2 * G + upto] if upto < G else w_cp[G - 1])
            if cold:
                launch(1)
            return proj_qk(b, g, w, o, MC, tk)

        def v_task(tk, g, t):
            y = proj_v(b, g, t, tk)
            if cold and t == 0 and g + 1 < G:
                transpose_wv(g + 1)
            return y

        def ln_task(tk, o):
            if cold and o == 0:
                arrive(x_cp[2])
            return ln_in(nxt, o, 16, tk)

        mm = []
        for g in range(G):
            for t in range(nq):
                for which in (1, 0):
                    for off in range(0, 128, MC):
                        mm.append(lambda tk, g=g, w=which, o=128 * t + off: qk_task(tk, g, w, o))
                        mm.extend([None] * (MC // 64 - 1))
                mm.extend([lambda tk, g=g, t=t: v_task(tk, g, t), None])
        if not head:
            for off in range(0, TB, MC):
                for c in range(G):
                    mm.append(lambda tk, o=off, c=c: wo_mm(b - 1, o, MC, 128 * c, 128, tk))
                    mm.extend([None] * (MC // 64 - 1))
        rowwise = [lambda tk, o=o: ln_task(tk, o) for o in range(0, TB, 16)]
        if not head:
            eb = jnp.where(b >= 2, b - 2, NB)
            rowwise = [lambda tk, o=o: epilogue(eb, o, 16, b >= 2, tk) for o in range(0, TB, 16)] + rowwise

        never = zero_s[...]
        st = dict(slot=0, y=None, tok=None, due=[])

        def dense():
            if not mm:
                st["tok"] = None
                return
            f = mm.pop(0)
            st["slot"] += 1
            st["tok"] = None if st["y"] is None else (never, st["y"][0:8])
            if f is None:
                st["y"] = st["y"][st["y"].shape[0] - 8:]
                return
            due = None
            while st["due"] and st["due"][0][0] <= st["slot"]:
                v, store = st["due"].pop(0)[1]
                store()
                due = (never, after(v, due))
            st["y"] = f(due)

        def fill(extra=0):
            if rowwise:
                st["due"].append((st["slot"] + LAG + extra, rowwise.pop(0)(st["tok"])))

        for c in range(LEAD):
            dense()
            if c % 2 == 1 and not head:
                fill()
        late = []
        sc, linv = {}, {}
        for u in range(len(units) + 1):
            if u < len(units):
                g, a = units[u]
                sc[u] = [qk(b * nq + a, g, j, nprev[a], (u % 2) * 4 + j) for j in range(4)]
                linv[u] = []
            acc = None
            for c in range(6):
                dense()
                if u >= 1:
                    pg, pa = units[u - 1]
                    if c in PV[:nprev[pa] + 1]:
                        acc, v = pv(b * nq + pa, pg, nprev[pa], ((u - 1) % 2) * 4, PV.index(c), acc)
                        if c != PV[2]:
                            st["due"].insert(0, (0, (v, lambda: None)))
                    if c == PV[3]:
                        store = att_out(b * nq + pa, pg, acc, linv.pop(u - 1))
                        if pg == G - 1:
                            late.append(store)
                        else:
                            store()
                for j in range(4):
                    if u < len(units) and c == SM[j]:
                        linv[u].append(softmax(*sc[u][j], (u % 2) * 4 + j, st["tok"]))
                if c in FILL[u % len(FILL)] and (u >= 2 or not head):
                    fill()
        while mm or rowwise:
            dense()
            fill(2)
            dense()
        for _, (_, store) in st["due"]:
            store()
        for store in late:
            store()

    def tail():
        never = zero_s[...]
        rowwise = [(NB - 2, o) for o in range(0, TB, 16)]
        y, due, n = None, [], 0
        for off in range(0, TB, 64):
            for c0 in range(0, D, 256):
                tok = None if y is None else (never, y[0:8])
                wait = None
                while due and due[0][0] <= n:
                    v, store = due.pop(0)[1]
                    store()
                    wait = (never, after(v, wait))
                y = wo_mm(NB - 1, off, 64, c0, 256, wait)
                for _ in range(2):
                    if rowwise:
                        due.append((n + TLAG, epilogue(*rowwise.pop(0), 16, None, tok)))
                n += 1
            rowwise += [(NB - 1, off + o) for o in range(0, 64, 16)]
        due += [(0, epilogue(*r, 16)) for r in rowwise]
        for _, (_, store) in due:
            store()

    def routed_token():
        best, bidx = best_s[...], bidx_s[...]
        top = jnp.max(best, axis=0, keepdims=True)
        idx = jnp.min(jnp.where(best == top, bidx, S - 1))
        grp = pl.multiple_of((idx >> 4) << 4, 16)
        x1 = x1_s[pl.ds(grp, 16), :].astype(F32)
        xn = _layernorm(x1).astype(BF16)
        sel = lax.broadcasted_iota(I32, (16, D), 0) == (idx & 15)
        row = jnp.sum(jnp.where(sel, xn.astype(F32), 0.0), axis=0, keepdims=True)
        for c in range(G):
            col_s[pl.ds(c * 128, 128), :] = jnp.broadcast_to(row[:, c * 128:(c + 1) * 128], (128, 128)).T

        y, hid = None, []
        for c in range(F // 256 + DLAG):
            if c < F // 256:
                wg = jnp.concatenate([wg_s.bitcast(I32)[2 * c + n] for n in range(2)], axis=1)
                gate = _rb(jnp.dot(xn, _bf(wg), preferred_element_type=F32))
                up = [0.0, 0.0]
                for r in range(0, D, 16):
                    col = col_s[pl.ds(r, 16), :]
                    for n in range(2):
                        w = _bf(wu_s.bitcast(I32)[2 * c + n, pl.ds(r // 2, 8), :]).astype(F32)
                        up[n] = up[n] + w * col
                up = _rb(jnp.sum(jnp.concatenate(up, axis=1), axis=0, keepdims=True))
                hid.append((_rb(gate * jax.nn.sigmoid(gate)) * up).astype(BF16))
            if c >= DLAG:
                r = pl.ds((c - DLAG) * 128, 128)
                wd = jnp.concatenate([wd_s.bitcast(I32)[n, r, :] for n in range(G)], axis=1)
                part = jnp.dot(hid[c - DLAG], _bf(wd), preferred_element_type=F32)
                y = part if y is None else y + part
        y = _rb(y)
        y = _rb(y * _rb(jax.nn.sigmoid(top[:, 0:1])))
        xn = xn.astype(F32)
        zero = xn * 0.0
        x2 = (x1 + _rb(xn + jnp.where(sel, zero + y, zero))).astype(BF16)
        return grp, x2

    launch()
    zero_s[...] = jnp.zeros((8, 128), I32)
    x1_s[rows(NB), :] = jnp.zeros((TB, D), BF16)
    for c in range(TB // 64):
        arrive(x_cp[c // 2])
        ln_in(0, 64 * c, 64)[1]()
    transpose_wv(0)
    body(0, True, cold=True)
    arrive(queue[-1])
    x_cp[4].start()

    def layer(li, carry):
        best_s[...] = jnp.full((8, 128), -jnp.inf, F32)
        bidx_s[...] = jnp.zeros((8, 128), I32)

        def step(b, c):
            body(b, False)

            @pl.when(jnp.logical_and(li == 0, b == 1))
            def _():
                x_cp[4].wait()
                for cp in ffn_cp:
                    cp.start()

            @pl.when(jnp.logical_and(li == 1, b >= 2))
            def _():
                out_cp(b - 2).start()
            return c

        lax.fori_loop(1, NB, step, 0)
        tail()

        @pl.when(li == 0)
        def _():
            for cp in ffn_cp:
                cp.wait()

        @pl.when(li == 1)
        def _():
            out_cp(NB - 2).start()
            out_cp(NB - 1).start()

        grp, x2 = routed_token()

        @pl.when(li == 0)
        def _():
            x_s[pl.ds(grp, 16), :] = x2
            xn = _layernorm(x2.astype(F32)).astype(BF16)
            for g in range(G):
                xn_s[g][pl.ds(grp, 16), :] = xn[:, g * 128:(g + 1) * 128]
            body(0, True)

        @pl.when(li == 1)
        def _():
            for blk in range(NB):
                out_cp(blk).wait()
            x_s[pl.ds(grp, 16), :] = x2
            cp = pltpu.make_async_copy(x_s.at[pl.ds(grp, 16)], out_hbm.at[pl.ds(grp, 16)], sem_o.at[0])
            cp.start()
            cp.wait()

        return carry

    lax.fori_loop(0, 2, layer, 0)


@jax.jit
def pallas_interleave_layers__sliding_block__moe_arch_mod__prompt_kernel(
    A_x: jax.Array,
    A_wqkv: jax.Array,
    A_wo: jax.Array,
    B_x: jax.Array,
    B_w_r: jax.Array,
    B_w_gate: jax.Array,
    B_w_up: jax.Array,
    B_w_down: jax.Array,
):
    del B_x
    hbm = pl.BlockSpec(memory_space=pl.ANY)
    out = pl.pallas_call(
        _kernel,
        out_shape=jax.ShapeDtypeStruct((S, D), BF16),
        in_specs=[hbm, hbm, hbm, pl.BlockSpec(memory_space=pltpu.VMEM), hbm, hbm, hbm],
        out_specs=hbm,
        scratch_shapes=[
            pltpu.VMEM((S + TB, D), BF16),
            pltpu.VMEM((S + TB, D), BF16),
            [pltpu.VMEM((S, 128), BF16)] * G,
            [pltpu.VMEM((S, 128), BF16)] * G,
            [pltpu.VMEM((S, 128), BF16)] * G,
            [pltpu.VMEM((S, 128), BF16)] * G,
            [pltpu.VMEM((S // 2, 128), I32)] * G,
            [pltpu.VMEM((256, 128), BF16)] * 8,
            [pltpu.VMEM((256, 128), BF16)] * 8,
            [pltpu.VMEM((D, 128), BF16)] * (3 * G),
            [pltpu.VMEM((D, 128), BF16)] * G,
            [pltpu.VMEM((D, 128), BF16)] * G,
            pltpu.VMEM((F // 128, D, 128), BF16),
            pltpu.VMEM((F // 128, D, 128), BF16),
            pltpu.VMEM((G, F, 128), BF16),
            pltpu.VMEM((8, 128), F32),
            pltpu.VMEM((8, 128), I32),
            pltpu.VMEM((8, 128), I32),
            pltpu.VMEM((D, 128), F32),
            pltpu.SemaphoreType.DMA((5,)),
            pltpu.SemaphoreType.DMA((4 * G,)),
            pltpu.SemaphoreType.DMA((1,)),
            pltpu.SemaphoreType.DMA((1,)),
        ],
        compiler_params=pltpu.CompilerParams(vmem_limit_bytes=100 * 1024 * 1024),
    )(A_x.reshape(S, D), A_wqkv, A_wo, B_w_r, B_w_gate, B_w_up, B_w_down)
    return out.reshape(1, S, D)
```
